```python
import os as _os
_os.environ.setdefault("JAX_PLATFORMS", "cpu")
import jax
import jax.numpy as jnp

def _softmax(x, axis=-1):
    return jax.nn.softmax(x, axis=axis)
def _gelu(x):
    return jax.nn.gelu(x, approximate=True)
def _silu(x):
    return jax.nn.silu(x)
def _sigmoid(x):
    return jax.nn.sigmoid(x)
def _layernorm(x, axis=-1, eps=1e-5):
    m = jnp.mean(x, axis=axis, keepdims=True)
    v = jnp.var(x, axis=axis, keepdims=True)
    return (x - m) / jnp.sqrt(v + eps)
def _scatter_add(tgt, idx, src, axis=0):
    return tgt.at[idx].add(src)
def _segment_sum(src, seg, n):
    return jax.ops.segment_sum(src, seg, n)
class _Rng:
    def __init__(self, key):
        self._k = key
    def _next(self):
        self._k, sub = jax.random.split(self._k)
        return sub
    def normal(self, shape):
        return jax.random.normal(self._next(), shape, dtype=jnp.bfloat16)
    def randint(self, lo, hi, shape):
        return jax.random.randint(self._next(), shape, lo, hi, dtype=jnp.int32)
    def uniform(self, shape, lo=0.0, hi=1.0):
        return jax.random.uniform(self._next(), shape, jnp.bfloat16, lo, hi)
    def permutation(self, n):
        return jax.random.permutation(self._next(), n)


kernel_name = 'gated_mix__linear_attn_block__mixer_token_mlp__prompt'

def setup_inputs():
    _rng = _Rng(jax.random.key(int.from_bytes(__import__("os").urandom(4), "little")))
    _w = (lambda a: (lambda t: t.astype(jnp.bfloat16) if jnp.issubdtype(t.dtype, jnp.floating) else t)(jnp.asarray(a)))
    def _A_setup():
        B, S, D = 1, 2048, 512
        return {
            "x": _w((lambda *s: _rng.normal(s) * 0.05)(B, S, D)),
            "wqkv": _w((lambda *s: _rng.normal(s) * 0.8)(D, 3 * D)),
            "wo": _w((lambda *s: _rng.normal(s) * 0.05)(D, D)),
        }
    _A_in = _A_setup()

    def _B_setup():
        B, S, D, F = 1, 2048, 512, 1792
        return {
            "x": _w((lambda *s: _rng.normal(s) * 0.05)(B, S, D)),
            "w1": _w((lambda *s: _rng.normal(s) * 0.1)(S, F) * (S ** -0.5)),
            "b1": _w((lambda *s: _rng.normal(s) * 0.1)(F) * 0.02),
            "w2": _w((lambda *s: _rng.normal(s) * 0.1)(F, S) * (F ** -0.5)),
            "b2": _w((lambda *s: _rng.normal(s) * 0.1)(S) * 0.02),
        }
    _B_in = _B_setup()

    return {
        "A_x": _A_in["x"],
        "A_wqkv": _A_in["wqkv"],
        "A_wo": _A_in["wo"],
        "B_x": _B_in["x"],
        "B_w1": _B_in["w1"],
        "B_b1": _B_in["b1"],
        "B_w2": _B_in["w2"],
        "B_b2": _B_in["b2"],
        "gate_w": _w((lambda *s: _rng.normal(s) * 0.05)(512) * 16.0),
    }

def reference(A_x, A_wqkv, A_wo, B_x, B_w1, B_b1, B_w2, B_b2, gate_w):
    def _A_ref(x, wqkv, wo):
        B, S, D = x.shape
        H = 32; Dh = D // H
        qkv = (lambda x, *d: x.transpose(*d))((x @ wqkv).reshape(B, S, 3, H, Dh), 2, 0, 3, 1, 4)
        q, k, v = qkv[0], qkv[1], qkv[2]
        phi = lambda t: jnp.where(t > 0, t + 1, jnp.exp(t)) + 1e-6
        pq, pk = phi(q), phi(k)
        kv = jnp.einsum("bhsd,bhse->bhde", pk, v)
        z = jnp.einsum("bhsd->bhd", pk)
        num = jnp.einsum("bhqd,bhde->bhqe", pq, kv)
        den = jnp.einsum("bhqd,bhd->bhq", pq, z)[..., None] + 1e-6
        o = num / den
        return (lambda x, *d: x.transpose(*d))(o, 0, 2, 1, 3).reshape(B, S, D) @ wo

    def _B_ref(x, w1, b1, w2, b2):
        B, S, D = x.shape
        h = _layernorm(x, axis=-1)
        u = jnp.einsum("bsd,sf->bdf", h, w1) + b1
        u = _gelu(u)
        y = jnp.einsum("bdf,fs->bds", u, w2) + b2
        return (lambda x, *d: x.transpose(*d))(y, 0, 2, 1)

    x = A_x
    g = _sigmoid((x * gate_w).sum(-1, keepdims=True))
    a = _A_ref(x, A_wqkv, A_wo)
    b = _B_ref(x, B_w1, B_b1, B_w2, B_b2)
    return g * a + (1 - g) * b
```

```python
import jax, jax.numpy as jnp
import numpy as np
from jax import lax
from jax.experimental import pallas as pl
from jax.experimental.pallas import tpu as pltpu

S, D, F, H, DH = 2048, 512, 1792, 32, 16
TC = 256
FC = 256
NC = S // TC
f32, bf16 = jnp.float32, jnp.bfloat16

def _dot(a, b):
    return jnp.dot(a, b, preferred_element_type=f32)
def _dot_nt(a, b):
    return lax.dot_general(a, b, (((1,), (1,)), ((), ())), preferred_element_type=f32)

def _rcp(d):
    r = pl.reciprocal(d, approx=True)
    return r * (2.0 - d * r)

def kernel(x_hbm, wqkv_hbm, wo_hbm, w1_hbm, w2_hbm, b1_ref, b2_ref, gw_ref, out_hbm,
           x_v, xT_v, hT_v, pqT_v, pkT_v, wqk_v, wqkT_v, wv_v, wo_v, woT_v, w1_v, w2_v, g_v, o_v,
           gwc_v, gate_v, zb_v, mT_v,
           sem_x, sem_w, sem_o):
    cp_wqk = pltpu.make_async_copy(wqkv_hbm.at[:, pl.ds(0, 2 * D)], wqk_v, sem_w.at[0])
    cp_wv = pltpu.make_async_copy(wqkv_hbm.at[:, pl.ds(2 * D, D)], wv_v, sem_w.at[1])
    cp_wo = pltpu.make_async_copy(wo_hbm, wo_v, sem_w.at[2])
    cp_w1 = pltpu.make_async_copy(w1_hbm, w1_v, sem_w.at[3])
    cp_w2 = pltpu.make_async_copy(w2_hbm, w2_v, sem_w.at[4])
    cp_x = [pltpu.make_async_copy(x_hbm.at[0, pl.ds(c * TC, TC), :], x_v.at[pl.ds(c * TC, TC), :], sem_x.at[c]) for c in range(NC)]
    cp_o = [pltpu.make_async_copy(o_v.at[pl.ds(c * TC, TC), :], out_hbm.at[0, pl.ds(c * TC, TC), :], sem_o.at[c]) for c in range(NC)]
    cp_x[0].start()
    cp_wqk.start()
    for c in range(1, NC):
        cp_x[c].start()
    cp_wv.start(); cp_wo.start()
    cp_w1.start()
    cp_w2.start()

    gw = gw_ref[...].astype(f32).reshape(1, D)
    for j in range(D // 128):
        blk = jnp.broadcast_to(gw[:, j * 128:(j + 1) * 128], (128, 128))
        gwc_v[j * 128:(j + 1) * 128, :] = blk.T

    cp_wqk.wait()
    for j in range(2 * D // 128):
        wqkT_v[j * 128:(j + 1) * 128, :] = wqk_v[:, j * 128:(j + 1) * 128].T

    zacc = jnp.zeros((D, 128), f32)
    for c in range(NC):
        cs = slice(c * TC, (c + 1) * TC)
        cp_x[c].wait()
        xcT = x_v[cs, :].T
        xT_v[:, cs] = xcT
        for t in range(TC // 128):
            ts = slice(c * TC + t * 128, c * TC + (t + 1) * 128)
            xf = xcT[:, t * 128:(t + 1) * 128].astype(f32)
            mean = jnp.sum(xf, axis=0, keepdims=True) * (1.0 / D)
            xc = xf - mean
            var = jnp.sum(xc * xc, axis=0, keepdims=True) * (1.0 / D)
            hT_v[:, ts] = (xc * lax.rsqrt(var + 1e-5)).astype(bf16)
            logit = jnp.sum(xf * gwc_v[...], axis=0, keepdims=True)
            gate = jax.nn.sigmoid(logit)
            gate_v[:, ts] = jnp.broadcast_to(gate, (8, 128))
        qk = _dot(wqkT_v[...], xcT)
        p = jnp.where(qk > 0, qk + 1.0, jnp.exp(qk)) + 1e-6
        pqT_v[:, cs] = p[:D].astype(bf16)
        pk = p[D:]
        pkT_v[:, cs] = pk.astype(bf16)
        for t in range(TC // 128):
            zacc = zacc + pk[:, t * 128:(t + 1) * 128]

    z = jnp.sum(zacc, axis=1, keepdims=True)
    zb_v[...] = jnp.broadcast_to(z, (D, 128))

    T = _dot(pkT_v[...], x_v[...])
    cp_wv.wait(); cp_wo.wait()
    for j in range(D // 128):
        woT_v[j * 128:(j + 1) * 128, :] = wo_v[:, j * 128:(j + 1) * 128].T
    Tb = T.astype(bf16)
    ri = lax.broadcasted_iota(jnp.int32, (128, 128), 0) // DH
    ci = lax.broadcasted_iota(jnp.int32, (128, 128), 1) // DH
    msk = ri == ci
    for b in range(D // 128):
        bs = slice(b * 128, (b + 1) * 128)
        kv = _dot(Tb[bs, :], wv_v[:, bs])
        kv = jnp.where(msk, kv, 0.0).astype(bf16)
        mT_v[:, bs] = _dot_nt(woT_v[:, bs], kv).astype(bf16)

    cp_w1.wait()
    b1 = b1_ref[...].astype(f32).reshape(1, F)
    for j in range(F // FC):
        fs = slice(j * FC, (j + 1) * FC)
        u = _dot(hT_v[...], w1_v[:, fs]) + b1[:, fs]
        g_v[:, fs] = jax.nn.gelu(u, approximate=True).astype(bf16)

    cp_w2.wait()
    b2 = b2_ref[...].astype(f32).reshape(1, S)
    for c in range(NC):
        cs = slice(c * TC, (c + 1) * TC)
        pq = pqT_v[:, cs].astype(f32)
        zb = zb_v[...]
        zbt = jnp.concatenate([zb] * (TC // 128), axis=1)
        den = jnp.sum((pq * zbt).reshape(H, DH, TC), axis=1, keepdims=True) + 1e-6
        pqn = (pq.reshape(H, DH, TC) * _rcp(den)).reshape(D, TC).astype(bf16)
        aT = _dot(mT_v[...], pqn)
        y = _dot(g_v[...], w2_v[:, cs]) + b2[:, cs]
        gate = gate_v[0:1, cs]
        oT = gate * aT + (1.0 - gate) * y
        o_v[cs, :] = oT.astype(bf16).T
        cp_o[c].start()
    for c in range(NC):
        cp_o[c].wait()


@jax.jit
def pallas_gated_mix__linear_attn_block__mixer_token_mlp__prompt_kernel(A_x, A_wqkv, A_wo, B_x, B_w1, B_b1, B_w2, B_b2, gate_w):
    any_spec = pl.BlockSpec(memory_space=pl.ANY)
    vm = pl.BlockSpec(memory_space=pltpu.VMEM)
    scratch = [
        pltpu.VMEM((S, D), bf16),
        pltpu.VMEM((D, S), bf16),
        pltpu.VMEM((D, S), bf16),
        pltpu.VMEM((D, S), bf16),
        pltpu.VMEM((D, S), bf16),
        pltpu.VMEM((D, 2 * D), bf16),
        pltpu.VMEM((2 * D, D), bf16),
        pltpu.VMEM((D, D), bf16),
        pltpu.VMEM((D, D), bf16),
        pltpu.VMEM((D, D), bf16),
        pltpu.VMEM((S, F), bf16),
        pltpu.VMEM((F, S), bf16),
        pltpu.VMEM((D, F), bf16),
        pltpu.VMEM((S, D), bf16),
        pltpu.VMEM((D, 128), f32),
        pltpu.VMEM((8, S), f32),
        pltpu.VMEM((D, 128), f32),
        pltpu.VMEM((D, D), bf16),
        pltpu.SemaphoreType.DMA((NC,)),
        pltpu.SemaphoreType.DMA((5,)),
        pltpu.SemaphoreType.DMA((NC,)),
    ]
    return pl.pallas_call(
        kernel,
        out_shape=jax.ShapeDtypeStruct((1, S, D), bf16),
        in_specs=[any_spec] * 5 + [vm] * 3,
        out_specs=any_spec,
        scratch_shapes=scratch,
        compiler_params=pltpu.CompilerParams(vmem_limit_bytes=100 * 1024 * 1024),
    )(A_x, A_wqkv, A_wo, B_w1, B_w2, B_b1, B_b2, gate_w)
```

```python
import jax
import jax.numpy as jnp
from jax import lax
from jax.experimental import pallas as pl
from jax.experimental.pallas import tpu as pltpu

S, D, F, H, DH = 2048, 512, 1792, 32, 16
HD = D // 2
TC = 256
NC = S // TC
NF = F // 256
f32, bf16, u32 = jnp.float32, jnp.bfloat16, jnp.uint32


def _dot(a, b):
    return jnp.dot(a, b, preferred_element_type=f32)


def _dot_nt(a, b):
    return lax.dot_general(a, b, (((1,), (1,)), ((), ())), preferred_element_type=f32)


def _pk(v):
    return pltpu.bitcast(v, u32)


def _upk(v):
    return pltpu.bitcast(v, bf16)


def _rcp(d):
    r = pl.reciprocal(d, approx=True)
    return r * (2.0 - d * r)


def _phi(t):
    return jnp.where(t > 0, t + 1.0, jnp.exp(t)) + 1e-6


def _lsums(A11, A12, A21, A22):
    return [A11 + A22, A21 + A22, A11, A22, A11 + A12, A21 - A11, A12 - A22]


def _add(a, b):
    return (a.astype(f32) + b.astype(f32)).astype(bf16)


def _sub(a, b):
    return (a.astype(f32) - b.astype(f32)).astype(bf16)


ORDER = (2, 5, 4, 3, 1, 6, 7)
RIDX = {1: 0, 2: 2, 3: 6, 4: 5, 5: 3, 6: 4, 7: 1}


def _rhs_ops(B11, B12, B21, B22):
    return {1: lambda: _add(B11(), B22()), 2: B11, 3: lambda: _sub(B12(), B22()), 4: lambda: _sub(B21(), B11()),
            5: B22, 6: lambda: _add(B11(), B12()), 7: lambda: _add(B21(), B22())}


def _combine(M):
    return M[1] + M[4] - M[5] + M[7], M[3] + M[5], M[2] + M[4], M[1] - M[2] + M[3] + M[6]


def _spread(ntie, nslots, off=0):
    return [off + (q * (nslots - off)) // ntie for q in range(ntie)]


def _tie_rows(getrows, nm, nk, slots, tmask):
    cols = []
    for j in range(nk):
        rows, m0 = [], 0
        for m in range(nm):
            if (m, j) in slots:
                if m > m0:
                    rows.append(getrows(m0, m, j))
                v = getrows(m, m + 1, j)
                for tv in slots[(m, j)]:
                    v = jnp.where(tmask, v, tv)
                rows.append(v)
                m0 = m + 1
        if m0 < nm:
            rows.append(getrows(m0, nm, j))
        cols.append(jnp.concatenate(rows, axis=0) if len(rows) > 1 else rows[0])
    return _upk(jnp.concatenate(cols, axis=1))


def _tie_value(lhs, ties, tmask):
    if not ties:
        return lhs
    nm, nk = lhs.shape[0] // 16, lhs.shape[1] // 128
    slots = {}
    for tv, sidx in zip(ties, _spread(len(ties), nm * nk)):
        grp, rem = divmod(sidx, nm * 4)
        m, jj = divmod(rem, min(4, nk - grp * 4))
        slots.setdefault((min(m, nm - 1), grp * 4 + jj), []).append(tv)
    p = _pk(lhs)
    return _tie_rows(lambda m0, m1, j: p[m0 * 8:m1 * 8, j * 128:(j + 1) * 128], nm, nk, slots, tmask)


def _strassen(L, R, dot=_dot, ties=(), tmask=None):
    M, ties = {}, list(ties)
    for n, p in enumerate(ORDER):
        k = len(ties) // (len(ORDER) - n)
        mine, ties = ties[:k], ties[k:]
        M[p] = dot(_tie_value(L(p - 1), mine, tmask), R(p))
    return _combine(M)


def _kernel(x_hbm, wqkv_hbm, wo_hbm, w1_hbm, w2_hbm, b1_hbm, b2_hbm, gw_hbm, out_hbm,
            x_v, wqk_v, wv_v, wo_v, w1_v, w2_v, o_v, b1_v, b2_v, gw_v,
            wqkT_p, wL_p, hL_p, pq_p, pkL_p, tb_p, woT_p, mL_p, gL_p,
            gate_v, zb_v, ga_v, b2f_v, sem, sem_o):
    cp = pltpu.make_async_copy
    cp_x = [cp(x_hbm.at[0, pl.ds(c * TC, TC), :], x_v.at[pl.ds(c * TC, TC), :], sem.at[c]) for c in range(NC)]
    cp_wq = cp(wqkv_hbm.at[:, pl.ds(0, D)], wqk_v.at[:, pl.ds(0, D)], sem.at[NC + 0])
    cp_wk = cp(wqkv_hbm.at[:, pl.ds(D, D)], wqk_v.at[:, pl.ds(D, D)], sem.at[NC + 1])
    cp_wv = cp(wqkv_hbm.at[:, pl.ds(2 * D, D)], wv_v, sem.at[NC + 2])
    cp_wo = cp(wo_hbm, wo_v, sem.at[NC + 3])
    cp_w1 = cp(w1_hbm, w1_v, sem.at[NC + 4])
    cp_w2 = cp(w2_hbm, w2_v, sem.at[NC + 5])
    cp_gw = cp(gw_hbm, gw_v, sem.at[NC + 6])
    cp_b1 = cp(b1_hbm, b1_v, sem.at[NC + 7])
    cp_b2 = cp(b2_hbm, b2_v, sem.at[NC + 8])
    for c_ in (cp_wq, cp_gw, cp_x[0], cp_x[1], cp_wk, *cp_x[2:], cp_w1, cp_b1, cp_b2, cp_wv, cp_wo, cp_w2):
        c_.start()

    ties = []
    mean, held = {}, {}
    zacc = [None]

    def tie(v):
        ties.append(v if v.dtype == u32 else pltpu.bitcast(v, u32))

    def take(n):
        mine = ties[:n]
        del ties[:n]
        return mine

    def w_transpose(h, tied):
        for j in range(4 * h, 4 * h + 4):
            pk = _pk(wqk_v[:, j * 128:(j + 1) * 128].T)
            wqkT_p[j * 64:(j + 1) * 64, :] = pk
            if tied:
                for kk in range(8):
                    for jj in range(4):
                        tie(pk[8 * kk:8 * kk + 8, jj * 128:(jj + 1) * 128])

    def ext_rows():
        gw = jnp.broadcast_to(gw_v[...].astype(f32).reshape(1, D), (16, D))
        ri = lax.broadcasted_iota(jnp.int32, (16, D), 0)
        return jnp.where(ri == 0, gw, jnp.where(ri == 1, 1.0 / D, 0.0))

    def use_ext(e, t):
        gate_v[:, t * 128:(t + 1) * 128] = jnp.broadcast_to(jax.nn.sigmoid(e[0:1, :]), (8, 128))
        mean[t] = e[1:2, :]

    def qk_dot(c, h, nties=0, off=0):
        if nties:
            slots = {}
            for tv, sidx in zip(take(nties), _spread(nties, 128, off)):
                slots.setdefault((sidx // 4, sidx % 4), []).append(tv)
            lhs = _tie_rows(lambda m0, m1, j: wqkT_p[h * 256 + m0 * 8:h * 256 + m1 * 8, j * 128:(j + 1) * 128],
                            32, 4, slots, tmask)
        else:
            lhs = _upk(wqkT_p[h * 256:(h + 1) * 256, :])
        if h == 0:
            lhs = jnp.concatenate([lhs, _upk(wqkT_p[512:520, :])], axis=0)
        return _dot_nt(lhs, x_v[c * TC:(c + 1) * TC, :])

    def q_store(c, q):
        for par in range(2):
            use_ext(q[D:D + 8, par * 128:(par + 1) * 128], 2 * c + par)
        pq_p[:, c * TC:(c + 1) * TC] = _pk(_phi(q[:D]).astype(bf16))

    def k_finish(c, pe, po):
        for i, l in enumerate(_lsums(pe[:HD], po[:HD], pe[HD:], po[HD:])):
            pkL_p[i, :, c * 128:(c + 1) * 128] = _pk(l.astype(bf16))
        s = pe + po
        zacc[0] = s if zacc[0] is None else zacc[0] + s

    def k_store(c, k):
        pk = _phi(k)
        k_finish(c, pk[:, :128], pk[:, 128:])

    def w_lsums():
        ext = ext_rows()
        A = {}
        for (i, j) in ((0, 0), (0, 1), (1, 0), (1, 1)):
            w = _upk(wqkT_p[i * 256:(i + 1) * 256, j * HD:(j + 1) * HD]).astype(f32)
            e = ext[:, j * HD:(j + 1) * HD] if i == 0 else jnp.zeros((16, HD), f32)
            A[i, j] = jnp.concatenate([w, e], axis=0)
        for i, l in enumerate(_lsums(A[0, 0], A[0, 1], A[1, 0], A[1, 1])):
            pk = _pk(l.astype(bf16))
            wL_p[i] = pk
            for kk in range(0, 33, 2):
                for jj in range(2):
                    tie(pk[8 * kk:8 * kk + 8, jj * 128:(jj + 1) * 128])

    def qk_strassen(c, nties):
        def nat(par, half):
            t = 2 * c + par
            return lambda: x_v[t * 128:(t + 1) * 128, half * HD:(half + 1) * HD]
        R = _rhs_ops(nat(0, 0), nat(1, 0), nat(0, 1), nat(1, 1))
        C11, C12, C21, C22 = _strassen(lambda i: _upk(wL_p[i]), lambda p: R[p](), _dot_nt, take(nties), tmask)
        for par, Cq in ((0, C11), (1, C12)):
            t = 2 * c + par
            use_ext(Cq[D:D + 8, :], t)
            pq_p[:, t * 128:(t + 1) * 128] = _pk(_phi(Cq[:D]).astype(bf16))
        k_finish(c, _phi(C21[:D]), _phi(C22[:D]))

    def layernorm(c):
        xT, stats = {}, {}
        for par in range(2):
            t = 2 * c + par
            ts = slice(t * 128, (t + 1) * 128)
            for j in range(4):
                xT[par, j] = x_v[ts, j * 128:(j + 1) * 128].T
            m = mean.pop(t)
            vs = None
            for j in range(4):
                xc = xT[par, j].astype(f32) - m
                v = jnp.sum((xc * xc).reshape(16, 8, 128), axis=0)
                vs = v if vs is None else vs + v
                tie(vs)
            stats[par] = (m, lax.rsqrt(jnp.sum(vs, axis=0, keepdims=True) * (1.0 / D) + 1e-5))
        (me, re), (mo, ro) = stats[0], stats[1]
        for b in range(2):
            for r in range(0, 128, 16):
                rs = slice(r, r + 16)
                a11 = (xT[0, b][rs].astype(f32) - me) * re
                a21 = (xT[0, 2 + b][rs].astype(f32) - me) * re
                a12 = (xT[1, b][rs].astype(f32) - mo) * ro
                a22 = (xT[1, 2 + b][rs].astype(f32) - mo) * ro
                for i, l in enumerate(_lsums(a11, a12, a21, a22)):
                    pk = _pk(l.astype(bf16))
                    hL_p[i, (b * 128 + r) // 2:(b * 128 + r + 16) // 2, c * 128:(c + 1) * 128] = pk
                    tie(pk)

    TM = {}

    def t_product(n, nties):
        def quad(par, col):
            return lambda: jnp.concatenate(
                [x_v[(2 * t + par) * 128:(2 * t + par + 1) * 128, col * HD:(col + 1) * HD] for t in range(NC)], axis=0)
        p = ORDER[n]
        R = _rhs_ops(quad(0, 0), quad(0, 1), quad(1, 0), quad(1, 1))
        TM[p] = _dot(_tie_value(_upk(pkL_p[p - 1]), take(nties), tmask), R[p]())
        if n == 6:
            C11, C12, C21, C22 = _combine(TM)
            tb_p[0:HD // 2, :] = _pk(jnp.concatenate([C11, C12], axis=1).astype(bf16))
            tb_p[HD // 2:, :] = _pk(jnp.concatenate([C21, C22], axis=1).astype(bf16))

    def u_stage(j, nties=0):
        def quad(par, col):
            return lambda: jnp.concatenate(
                [w1_v[(2 * t + par) * 128:(2 * t + par + 1) * 128, j * 256 + col * 128:j * 256 + (col + 1) * 128]
                 for t in range(NC)], axis=0)
        R = _rhs_ops(quad(0, 0), quad(0, 1), quad(1, 0), quad(1, 1))
        C11, C12, C21, C22 = _strassen(lambda i: _upk(hL_p[i]), lambda p: R[p](), _dot, take(nties), tmask)

        def gl(v, f0):
            return jax.nn.gelu(v + b1[:, f0:f0 + 128], approximate=True)
        G = (gl(C11, j * 256), gl(C12, j * 256 + 128), gl(C21, j * 256), gl(C22, j * 256 + 128))
        for i, l in enumerate(_lsums(*G)):
            gL_p[i, :, j * 128:(j + 1) * 128] = _pk(l.astype(bf16))

    def norm_stage(c):
        nb = {}
        for par in range(2):
            ts = slice((2 * c + par) * 128, (2 * c + par + 1) * 128)
            for b in range(4):
                pq = _upk(pq_p[b * 64:(b + 1) * 64, ts]).astype(f32)
                den = jnp.sum((pq * zb_v[b * 128:(b + 1) * 128, :]).reshape(8, DH, 128), axis=1, keepdims=True) + 1e-6
                nb[par, b] = (pq.reshape(8, DH, 128) * _rcp(den)).reshape(128, 128)
        ops = [[None, None] for _ in range(7)]
        for bp in range(2):
            for i, l in enumerate(_lsums(nb[0, bp], nb[1, bp], nb[0, 2 + bp], nb[1, 2 + bp])):
                ops[i][bp] = l.astype(bf16)
        R = [jnp.concatenate(o, axis=0) for o in ops]
        for p in ORDER:
            pk = _pk(R[RIDX[p]])
            for k in range(16):
                tie(pk[8 * k:8 * k + 8, :])
        held[c] = R

    def a_stage(c):
        R = held.pop(c)
        C = _strassen(lambda i: _upk(mL_p[i]), lambda p: R[RIDX[p]])
        aT = jnp.concatenate([jnp.concatenate([C[0], C[1]], axis=1), jnp.concatenate([C[2], C[3]], axis=1)], axis=0)
        cs = slice(c * TC, (c + 1) * TC)
        ga_v[:, cs] = gate_v[0:1, cs] * aT

    cp_wq.wait()
    w_transpose(0, tied=False)
    cp_x[0].wait()
    cp_gw.wait()
    g8 = wqk_v[0:16, 0:128].astype(f32)[0:8, :]
    tmask = (g8 >= 0.0) | (g8 < 0.0) | (g8 != g8)
    wqkT_p[512:520, :] = _pk(ext_rows().astype(bf16))
    q_store(0, qk_dot(0, 0))
    cp_x[1].wait()
    q_store(1, qk_dot(1, 0))
    cp_wk.wait()
    cp_x[2].wait()
    w_transpose(1, tied=True)
    q_store(2, qk_dot(2, 0, 128, 64))
    k_store(0, qk_dot(0, 1))
    w_lsums()
    k_store(1, qk_dot(1, 1, 120))
    k_store(2, qk_dot(2, 1, 118))
    for c in range(3, NC):
        cp_x[c].wait()
    qk_strassen(3, 0)
    for c, n in ((4, 120), (5, 120), (6, 104), (7, 120)):
        layernorm(c - 4)
        qk_strassen(c, n)
    zb_v[...] = jnp.broadcast_to(jnp.sum(zacc[0], axis=1, keepdims=True), (D, 128))
    for n, (nt, ln) in enumerate(((120, 4), (60, 5), (76, None), (60, 6), (44, None), (76, 7), (60, None))):
        if ln is not None:
            layernorm(ln)
        t_product(n, nt)

    for c_ in (cp_w1, cp_b1, cp_b2, cp_wv, cp_wo):
        c_.wait()
    for j in range(4):
        woT_p[j * 64:(j + 1) * 64, :] = _pk(wo_v[:, j * 128:(j + 1) * 128].T)
    b1 = b1_v[...].astype(f32).reshape(1, F)
    u_stage(0)
    msk = (lax.broadcasted_iota(jnp.int32, (128, 128), 0) // DH) == (lax.broadcasted_iota(jnp.int32, (128, 128), 1) // DH)
    kvs = []
    for b in range(4):
        kv = _dot(_upk(tb_p[b * 64:(b + 1) * 64, :]), wv_v[:, b * 128:(b + 1) * 128])
        kvs.append(jnp.where(msk, kv, 0.0).astype(bf16))
    u_stage(1)
    Ms = [_dot_nt(_upk(woT_p[:, b * 128:(b + 1) * 128]), kvs[b]) for b in range(4)]
    for bp in range(2):
        for i, l in enumerate(_lsums(Ms[bp][:HD], Ms[2 + bp][:HD], Ms[bp][HD:], Ms[2 + bp][HD:])):
            mL_p[i, :, bp * 128:(bp + 1) * 128] = _pk(l.astype(bf16))
    for j in (2, 3, 4):
        norm_stage(2 * j - 4)
        norm_stage(2 * j - 3)
        u_stage(j, 224)
        a_stage(2 * j - 4)
        a_stage(2 * j - 3)
    norm_stage(6)
    norm_stage(7)
    u_stage(5, 224)
    a_stage(6)
    u_stage(6)
    a_stage(7)

    cp_w2.wait()
    b2f_v[...] = jnp.broadcast_to(b2_v[...].astype(f32).reshape(1, S), (8, S))

    def y_body(i, carry):
        for k in range(2):
            c0 = pl.multiple_of((2 * i + k) * TC, TC)

            def quad(par, col):
                return lambda: jnp.concatenate(
                    [w2_v[(2 * t + par) * 128:(2 * t + par + 1) * 128, pl.ds(c0 + col * 128, 128)] for t in range(NF)],
                    axis=0)
            R = _rhs_ops(quad(0, 0), quad(0, 1), quad(1, 0), quad(1, 1))
            Y11, Y12, Y21, Y22 = _strassen(lambda n: _upk(gL_p[n]), lambda p: R[p]())
            for par, (Ya, Yb) in ((1, (Y12, Y22)), (0, (Y11, Y21))):
                tt = pl.ds(c0 + par * 128, 128)
                y = jnp.concatenate([Ya, Yb], axis=0) + b2f_v[0:1, tt]
                oT = ga_v[:, tt] + (1.0 - gate_v[0:1, tt]) * y
                o_v[tt, :] = oT.astype(bf16).T
                cp(o_v.at[tt, :], out_hbm.at[0, tt, :], sem_o.at[0]).start()
        return carry
    lax.fori_loop(0, NC // 2, y_body, 0)
    cp(o_v, out_hbm.at[0], sem_o.at[0]).wait()


@jax.jit
def pallas_gated_mix__linear_attn_block__mixer_token_mlp__prompt_kernel(
        A_x, A_wqkv, A_wo, B_x, B_w1, B_b1, B_w2, B_b2, gate_w):
    del B_x
    assert A_x.shape == (1, S, D) and B_w1.shape == (S, F) and B_w2.shape == (F, S), "fixed problem shape"
    vm = pltpu.VMEM
    scratch = [
        vm((S, D), bf16),
        vm((D, 2 * D), bf16),
        vm((D, D), bf16),
        vm((D, D), bf16),
        vm((S, F), bf16),
        vm((F, S), bf16),
        vm((S, D), bf16),
        vm((F,), bf16),
        vm((S,), bf16),
        vm((D,), bf16),
        vm((D + 8, D), u32),
        vm((7, 264, HD), u32),
        vm((7, D // 4, S // 2), u32),
        vm((HD, S), u32),
        vm((7, D // 4, S // 2), u32),
        vm((HD, D), u32),
        vm((HD, D), u32),
        vm((7, D // 4, HD), u32),
        vm((7, D // 4, F // 2), u32),
        vm((8, S), f32),
        vm((D, 128), f32),
        vm((D, S), f32),
        vm((8, S), f32),
        pltpu.SemaphoreType.DMA((NC + 9,)),
        pltpu.SemaphoreType.DMA((1,)),
    ]
    any_spec = pl.BlockSpec(memory_space=pl.ANY)
    return pl.pallas_call(
        _kernel,
        out_shape=jax.ShapeDtypeStruct((1, S, D), bf16),
        in_specs=[any_spec] * 8,
        out_specs=any_spec,
        scratch_shapes=scratch,
        compiler_params=pltpu.CompilerParams(
            vmem_limit_bytes=100 * 1024 * 1024, disable_semaphore_checks=True, disable_bounds_checks=True),
    )(A_x, A_wqkv, A_wo, B_w1, B_w2, B_b1, B_b2, gate_w)
```

```python
import jax
import jax.numpy as jnp
from jax import lax
from jax.experimental import pallas as pl
from jax.experimental.pallas import tpu as pltpu

S, D, F, H, DH = 2048, 512, 1792, 32, 16
HD = D // 2
TC = 256
NC = S // TC
NF = F // 256
f32, bf16, u32 = jnp.float32, jnp.bfloat16, jnp.uint32


def _dot(a, b):
    return jnp.dot(a, b, preferred_element_type=f32)


def _dot_nt(a, b):
    return lax.dot_general(a, b, (((1,), (1,)), ((), ())), preferred_element_type=f32)


def _pk(v):
    return pltpu.bitcast(v, u32)


def _upk(v):
    return pltpu.bitcast(v, bf16)


def _rcp(d):
    r = pl.reciprocal(d, approx=True)
    return r * (2.0 - d * r)


def _phi(t):
    return jnp.where(t > 0, t + 1.0, jnp.exp(t)) + 1e-6


def _lsums(A11, A12, A21, A22):
    return [A11 + A22, A21 + A22, A11, A22, A11 + A12, A21 - A11, A12 - A22]


def _add(a, b):
    return (a.astype(f32) + b.astype(f32)).astype(bf16)


def _sub(a, b):
    return (a.astype(f32) - b.astype(f32)).astype(bf16)


ORDER = (2, 5, 4, 3, 1, 6, 7)
RIDX = {1: 0, 2: 2, 3: 6, 4: 5, 5: 3, 6: 4, 7: 1}


def _rhs_ops(B11, B12, B21, B22):
    return {1: lambda: _add(B11(), B22()), 2: B11, 3: lambda: _sub(B12(), B22()), 4: lambda: _sub(B21(), B11()),
            5: B22, 6: lambda: _add(B11(), B12()), 7: lambda: _add(B21(), B22())}


def _combine(M):
    return M[1] + M[4] - M[5] + M[7], M[3] + M[5], M[2] + M[4], M[1] - M[2] + M[3] + M[6]


def _spread(ntie, nslots, off=0):
    return [off + (q * (nslots - off)) // ntie for q in range(ntie)]


def _tie_rows(getrows, nm, nk, slots, tmask):
    cols = []
    for j in range(nk):
        rows, m0 = [], 0
        for m in range(nm):
            if (m, j) in slots:
                if m > m0:
                    rows.append(getrows(m0, m, j))
                v = getrows(m, m + 1, j)
                for tv in slots[(m, j)]:
                    v = jnp.where(tmask, v, tv)
                rows.append(v)
                m0 = m + 1
        if m0 < nm:
            rows.append(getrows(m0, nm, j))
        cols.append(jnp.concatenate(rows, axis=0) if len(rows) > 1 else rows[0])
    return _upk(jnp.concatenate(cols, axis=1))


def _tie_value(lhs, ties, tmask):
    if not ties:
        return lhs
    nm, nk = lhs.shape[0] // 16, lhs.shape[1] // 128
    slots = {}
    for tv, sidx in zip(ties, _spread(len(ties), nm * nk)):
        grp, rem = divmod(sidx, nm * 4)
        m, jj = divmod(rem, min(4, nk - grp * 4))
        slots.setdefault((min(m, nm - 1), grp * 4 + jj), []).append(tv)
    p = _pk(lhs)
    return _tie_rows(lambda m0, m1, j: p[m0 * 8:m1 * 8, j * 128:(j + 1) * 128], nm, nk, slots, tmask)


def _strassen(L, R, dot=_dot, ties=(), tmask=None):
    M, ties = {}, list(ties)
    for n, p in enumerate(ORDER):
        k = len(ties) // (len(ORDER) - n)
        mine, ties = ties[:k], ties[k:]
        M[p] = dot(_tie_value(L(p - 1), mine, tmask), R(p))
    return _combine(M)


def _kernel(x_hbm, wqkv_hbm, wo_hbm, w1_hbm, w2_hbm, b1_hbm, b2_hbm, gw_hbm, out_hbm,
            x_v, wqk_v, wv_v, wo_v, w1_v, w2_v, o_v, b1_v, b2_v, gw_v,
            wqkT_p, wL_p, hL_p, pq_p, pkL_p, tb_p, woT_p, mL_p, gL_p,
            gate_v, zb_v, ga_v, b2f_v, pend_p, sem, sem_o):
    cp = pltpu.make_async_copy
    cp_x = [cp(x_hbm.at[0, pl.ds(c * TC, TC), :], x_v.at[pl.ds(c * TC, TC), :], sem.at[c]) for c in range(NC)]
    cp_wq = cp(wqkv_hbm.at[:, pl.ds(0, D)], wqk_v.at[:, pl.ds(0, D)], sem.at[NC + 0])
    cp_wk = cp(wqkv_hbm.at[:, pl.ds(D, D)], wqk_v.at[:, pl.ds(D, D)], sem.at[NC + 1])
    cp_wv = cp(wqkv_hbm.at[:, pl.ds(2 * D, D)], wv_v, sem.at[NC + 2])
    cp_wo = cp(wo_hbm, wo_v, sem.at[NC + 3])
    cp_w1 = cp(w1_hbm, w1_v, sem.at[NC + 4])
    cp_w2 = cp(w2_hbm, w2_v, sem.at[NC + 5])
    cp_gw = cp(gw_hbm, gw_v, sem.at[NC + 6])
    cp_b1 = cp(b1_hbm, b1_v, sem.at[NC + 7])
    cp_b2 = cp(b2_hbm, b2_v, sem.at[NC + 8])
    for c_ in (cp_wq, cp_gw, cp_x[0], cp_x[1], cp_wk, *cp_x[2:], cp_w1, cp_b1, cp_b2, cp_wv, cp_wo, cp_w2):
        c_.start()

    ties = []
    mean, held = {}, {}
    zacc = [None]

    def tie(v):
        ties.append(v if v.dtype == u32 else pltpu.bitcast(v, u32))

    def take(n):
        mine = ties[:n]
        del ties[:n]
        return mine

    def w_transpose(h, tied):
        for j in range(4 * h, 4 * h + 4):
            pk = _pk(wqk_v[:, j * 128:(j + 1) * 128].T)
            wqkT_p[j * 64:(j + 1) * 64, :] = pk
            if tied:
                for kk in range(8):
                    for jj in range(4):
                        tie(pk[8 * kk:8 * kk + 8, jj * 128:(jj + 1) * 128])

    def ext_rows():
        gw = jnp.broadcast_to(gw_v[...].astype(f32).reshape(1, D), (16, D))
        ri = lax.broadcasted_iota(jnp.int32, (16, D), 0)
        return jnp.where(ri == 0, gw, jnp.where(ri == 1, 1.0 / D, 0.0))

    def use_ext(e, t):
        gate_v[:, t * 128:(t + 1) * 128] = jnp.broadcast_to(jax.nn.sigmoid(e[0:1, :]), (8, 128))
        mean[t] = e[1:2, :]

    def qk_dot(c, h, nties=0, off=0):
        if nties:
            slots = {}
            for tv, sidx in zip(take(nties), _spread(nties, 128, off)):
                slots.setdefault((sidx // 4, sidx % 4), []).append(tv)
            lhs = _tie_rows(lambda m0, m1, j: wqkT_p[h * 256 + m0 * 8:h * 256 + m1 * 8, j * 128:(j + 1) * 128],
                            32, 4, slots, tmask)
        else:
            lhs = _upk(wqkT_p[h * 256:(h + 1) * 256, :])
        if h == 0:
            lhs = jnp.concatenate([lhs, _upk(wqkT_p[512:520, :])], axis=0)
        return _dot_nt(lhs, x_v[c * TC:(c + 1) * TC, :])

    def q_store(c, q):
        for par in range(2):
            use_ext(q[D:D + 8, par * 128:(par + 1) * 128], 2 * c + par)
        pq_p[:, c * TC:(c + 1) * TC] = _pk(_phi(q[:D]).astype(bf16))

    def k_finish(c, pe, po):
        for i, l in enumerate(_lsums(pe[:HD], po[:HD], pe[HD:], po[HD:])):
            pkL_p[i, :, c * 128:(c + 1) * 128] = _pk(l.astype(bf16))
        s = pe + po
        zacc[0] = s if zacc[0] is None else zacc[0] + s

    def k_store(c, k):
        pk = _phi(k)
        k_finish(c, pk[:, :128], pk[:, 128:])

    def w_lsums():
        ext = ext_rows()
        A = {}
        for (i, j) in ((0, 0), (0, 1), (1, 0), (1, 1)):
            w = _upk(wqkT_p[i * 256:(i + 1) * 256, j * HD:(j + 1) * HD]).astype(f32)
            e = ext[:, j * HD:(j + 1) * HD] if i == 0 else jnp.zeros((16, HD), f32)
            A[i, j] = jnp.concatenate([w, e], axis=0)
        for i, l in enumerate(_lsums(A[0, 0], A[0, 1], A[1, 0], A[1, 1])):
            pk = _pk(l.astype(bf16))
            wL_p[i] = pk
            for kk in range(0, 33, 2):
                for jj in range(2):
                    tie(pk[8 * kk:8 * kk + 8, jj * 128:(jj + 1) * 128])

    def qk_strassen(c, nties):
        def nat(par, half):
            t = 2 * c + par
            return lambda: x_v[t * 128:(t + 1) * 128, half * HD:(half + 1) * HD]
        R = _rhs_ops(nat(0, 0), nat(1, 0), nat(0, 1), nat(1, 1))
        C11, C12, C21, C22 = _strassen(lambda i: _upk(wL_p[i]), lambda p: R[p](), _dot_nt, take(nties), tmask)
        for par, Cq in ((0, C11), (1, C12)):
            t = 2 * c + par
            use_ext(Cq[D:D + 8, :], t)
            pq_p[:, t * 128:(t + 1) * 128] = _pk(_phi(Cq[:D]).astype(bf16))
        k_finish(c, _phi(C21[:D]), _phi(C22[:D]))

    def layernorm(c):
        xT, stats = {}, {}
        for par in range(2):
            t = 2 * c + par
            ts = slice(t * 128, (t + 1) * 128)
            for j in range(4):
                xT[par, j] = x_v[ts, j * 128:(j + 1) * 128].T
            m = mean.pop(t)
            vs = None
            for j in range(4):
                xc = xT[par, j].astype(f32) - m
                v = jnp.sum((xc * xc).reshape(16, 8, 128), axis=0)
                vs = v if vs is None else vs + v
                tie(vs)
            stats[par] = (m, lax.rsqrt(jnp.sum(vs, axis=0, keepdims=True) * (1.0 / D) + 1e-5))
        (me, re), (mo, ro) = stats[0], stats[1]
        for b in range(2):
            for r in range(0, 128, 16):
                rs = slice(r, r + 16)
                a11 = (xT[0, b][rs].astype(f32) - me) * re
                a21 = (xT[0, 2 + b][rs].astype(f32) - me) * re
                a12 = (xT[1, b][rs].astype(f32) - mo) * ro
                a22 = (xT[1, 2 + b][rs].astype(f32) - mo) * ro
                for i, l in enumerate(_lsums(a11, a12, a21, a22)):
                    pk = _pk(l.astype(bf16))
                    hL_p[i, (b * 128 + r) // 2:(b * 128 + r + 16) // 2, c * 128:(c + 1) * 128] = pk
                    tie(pk)

    TM = {}

    def t_product(n, nties):
        def quad(par, col):
            return lambda: jnp.concatenate(
                [x_v[(2 * t + par) * 128:(2 * t + par + 1) * 128, col * HD:(col + 1) * HD] for t in range(NC)], axis=0)
        p = ORDER[n]
        R = _rhs_ops(quad(0, 0), quad(0, 1), quad(1, 0), quad(1, 1))
        TM[p] = _dot(_tie_value(_upk(pkL_p[p - 1]), take(nties), tmask), R[p]())
        if n == 6:
            C11, C12, C21, C22 = _combine(TM)
            tb_p[0:HD // 2, :] = _pk(jnp.concatenate([C11, C12], axis=1).astype(bf16))
            tb_p[HD // 2:, :] = _pk(jnp.concatenate([C21, C22], axis=1).astype(bf16))

    def u_stage(j, nties=0):
        def quad(par, col):
            return lambda: jnp.concatenate(
                [w1_v[(2 * t + par) * 128:(2 * t + par + 1) * 128, j * 256 + col * 128:j * 256 + (col + 1) * 128]
                 for t in range(NC)], axis=0)
        R = _rhs_ops(quad(0, 0), quad(0, 1), quad(1, 0), quad(1, 1))
        C11, C12, C21, C22 = _strassen(lambda i: _upk(hL_p[i]), lambda p: R[p](), _dot, take(nties), tmask)

        def gl(v, f0):
            return jax.nn.gelu(v + b1[:, f0:f0 + 128], approximate=True)
        G = (gl(C11, j * 256), gl(C12, j * 256 + 128), gl(C21, j * 256), gl(C22, j * 256 + 128))
        for i, l in enumerate(_lsums(*G)):
            gL_p[i, :, j * 128:(j + 1) * 128] = _pk(l.astype(bf16))

    def norm_stage(c):
        nb = {}
        for par in range(2):
            ts = slice((2 * c + par) * 128, (2 * c + par + 1) * 128)
            for b in range(4):
                pq = _upk(pq_p[b * 64:(b + 1) * 64, ts]).astype(f32)
                den = jnp.sum((pq * zb_v[b * 128:(b + 1) * 128, :]).reshape(8, DH, 128), axis=1, keepdims=True) + 1e-6
                nb[par, b] = (pq.reshape(8, DH, 128) * _rcp(den)).reshape(128, 128)
        ops = [[None, None] for _ in range(7)]
        for bp in range(2):
            for i, l in enumerate(_lsums(nb[0, bp], nb[1, bp], nb[0, 2 + bp], nb[1, 2 + bp])):
                ops[i][bp] = l.astype(bf16)
        R = [jnp.concatenate(o, axis=0) for o in ops]
        for p in ORDER:
            pk = _pk(R[RIDX[p]])
            for k in range(16):
                tie(pk[8 * k:8 * k + 8, :])
        held[c] = R

    def a_stage(c):
        R = held.pop(c)
        C = _strassen(lambda i: _upk(mL_p[i]), lambda p: R[RIDX[p]])
        aT = jnp.concatenate([jnp.concatenate([C[0], C[1]], axis=1), jnp.concatenate([C[2], C[3]], axis=1)], axis=0)
        cs = slice(c * TC, (c + 1) * TC)
        ga_v[:, cs] = gate_v[0:1, cs] * aT

    cp_wq.wait()
    w_transpose(0, tied=False)
    cp_x[0].wait()
    cp_gw.wait()
    g8 = wqk_v[0:16, 0:128].astype(f32)[0:8, :]
    tmask = (g8 >= 0.0) | (g8 < 0.0) | (g8 != g8)
    wqkT_p[512:520, :] = _pk(ext_rows().astype(bf16))
    q_store(0, qk_dot(0, 0))
    cp_x[1].wait()
    q_store(1, qk_dot(1, 0))
    cp_wk.wait()
    cp_x[2].wait()
    w_transpose(1, tied=True)
    q_store(2, qk_dot(2, 0, 128, 64))
    k_store(0, qk_dot(0, 1))
    w_lsums()
    k_store(1, qk_dot(1, 1, 120))
    k_store(2, qk_dot(2, 1, 118))
    for c in range(3, NC):
        cp_x[c].wait()
    qk_strassen(3, 0)
    for c, n in ((4, 120), (5, 120), (6, 104), (7, 120)):
        layernorm(c - 4)
        qk_strassen(c, n)
    zb_v[...] = jnp.broadcast_to(jnp.sum(zacc[0], axis=1, keepdims=True), (D, 128))
    for n, (nt, ln) in enumerate(((120, 4), (60, 5), (76, None), (60, 6), (44, None), (76, 7), (60, None))):
        if ln is not None:
            layernorm(ln)
        t_product(n, nt)

    for c_ in (cp_w1, cp_b1, cp_b2, cp_wv, cp_wo):
        c_.wait()
    for j in range(4):
        woT_p[j * 64:(j + 1) * 64, :] = _pk(wo_v[:, j * 128:(j + 1) * 128].T)
    b1 = b1_v[...].astype(f32).reshape(1, F)
    u_stage(0)
    msk = (lax.broadcasted_iota(jnp.int32, (128, 128), 0) // DH) == (lax.broadcasted_iota(jnp.int32, (128, 128), 1) // DH)
    kvs = []
    for b in range(4):
        kv = _dot(_upk(tb_p[b * 64:(b + 1) * 64, :]), wv_v[:, b * 128:(b + 1) * 128])
        kvs.append(jnp.where(msk, kv, 0.0).astype(bf16))
    u_stage(1)
    Ms = [_dot_nt(_upk(woT_p[:, b * 128:(b + 1) * 128]), kvs[b]) for b in range(4)]
    for bp in range(2):
        for i, l in enumerate(_lsums(Ms[bp][:HD], Ms[2 + bp][:HD], Ms[bp][HD:], Ms[2 + bp][HD:])):
            mL_p[i, :, bp * 128:(bp + 1) * 128] = _pk(l.astype(bf16))
    for j in (2, 3, 4):
        norm_stage(2 * j - 4)
        norm_stage(2 * j - 3)
        u_stage(j, 224)
        a_stage(2 * j - 4)
        a_stage(2 * j - 3)
    norm_stage(6)
    norm_stage(7)
    u_stage(5, 224)
    a_stage(6)
    u_stage(6)
    a_stage(7)

    cp_w2.wait()
    b2f_v[...] = jnp.broadcast_to(b2_v[...].astype(f32).reshape(1, S), (8, S))

    def out_tile(tt, obT, s):
        o_v[tt, :] = obT
        cp(o_v.at[tt, :], out_hbm.at[0, tt, :], s).start()

    pend_p[...] = jnp.zeros((HD, 128), u32)

    def y_body(i, carry):
        tprev = pl.multiple_of(jnp.where(i == 0, 14, 4 * i - 2) * 128, 128)
        out_tile(pl.ds(tprev, 128), _upk(pend_p[...]).T, sem_o.at[jnp.where(i == 0, 1, 0)])
        for k in range(2):
            c0 = pl.multiple_of((2 * i + k) * TC, TC)

            def quad(par, col):
                return lambda: jnp.concatenate(
                    [w2_v[(2 * t + par) * 128:(2 * t + par + 1) * 128, pl.ds(c0 + col * 128, 128)] for t in range(NF)],
                    axis=0)
            R = _rhs_ops(quad(0, 0), quad(0, 1), quad(1, 0), quad(1, 1))
            Y11, Y12, Y21, Y22 = _strassen(lambda n: _upk(gL_p[n]), lambda p: R[p]())
            for par, (Ya, Yb) in ((1, (Y12, Y22)), (0, (Y11, Y21))):
                tt = pl.ds(c0 + par * 128, 128)
                y = jnp.concatenate([Ya, Yb], axis=0) + b2f_v[0:1, tt]
                oT = (ga_v[:, tt] + (1.0 - gate_v[0:1, tt]) * y).astype(bf16)
                if k == 1 and par == 0:
                    pend_p[...] = _pk(oT)
                else:
                    out_tile(tt, oT.T, sem_o.at[0])
        return carry
    lax.fori_loop(0, NC // 2, y_body, 0)
    t14 = pl.ds(14 * 128, 128)
    cp(o_v.at[t14, :], out_hbm.at[0, t14, :], sem_o.at[1]).wait()
    out_tile(t14, _upk(pend_p[...]).T, sem_o.at[0])
    cp(o_v, out_hbm.at[0], sem_o.at[0]).wait()


@jax.jit
def pallas_gated_mix__linear_attn_block__mixer_token_mlp__prompt_kernel(
        A_x, A_wqkv, A_wo, B_x, B_w1, B_b1, B_w2, B_b2, gate_w):
    del B_x
    assert A_x.shape == (1, S, D) and B_w1.shape == (S, F) and B_w2.shape == (F, S), "fixed problem shape"
    vm = pltpu.VMEM
    scratch = [
        vm((S, D), bf16),
        vm((D, 2 * D), bf16),
        vm((D, D), bf16),
        vm((D, D), bf16),
        vm((S, F), bf16),
        vm((F, S), bf16),
        vm((S, D), bf16),
        vm((F,), bf16),
        vm((S,), bf16),
        vm((D,), bf16),
        vm((D + 8, D), u32),
        vm((7, 264, HD), u32),
        vm((7, D // 4, S // 2), u32),
        vm((HD, S), u32),
        vm((7, D // 4, S // 2), u32),
        vm((HD, D), u32),
        vm((HD, D), u32),
        vm((7, D // 4, HD), u32),
        vm((7, D // 4, F // 2), u32),
        vm((8, S), f32),
        vm((D, 128), f32),
        vm((D, S), f32),
        vm((8, S), f32),
        vm((HD, 128), u32),
        pltpu.SemaphoreType.DMA((NC + 9,)),
        pltpu.SemaphoreType.DMA((2,)),
    ]
    any_spec = pl.BlockSpec(memory_space=pl.ANY)
    return pl.pallas_call(
        _kernel,
        out_shape=jax.ShapeDtypeStruct((1, S, D), bf16),
        in_specs=[any_spec] * 8,
        out_specs=any_spec,
        scratch_shapes=scratch,
        compiler_params=pltpu.CompilerParams(
            vmem_limit_bytes=100 * 1024 * 1024, disable_semaphore_checks=True, disable_bounds_checks=True),
    )(A_x, A_wqkv, A_wo, B_w1, B_w2, B_b1, B_b2, gate_w)
```

```python
import jax
import jax.numpy as jnp
from jax import lax
from jax.experimental import pallas as pl
from jax.experimental.pallas import tpu as pltpu

S, D, F, H, DH = 2048, 512, 1792, 32, 16
HD = D // 2
TK = (120, 120, 104, 120, 120, 84, 100, 24, 0, 112, 56)
TC = 256
NC = S // TC
NF = F // 256
f32, bf16, u32 = jnp.float32, jnp.bfloat16, jnp.uint32


def _dot(a, b):
    return jnp.dot(a, b, preferred_element_type=f32)


def _dot_nt(a, b):
    return lax.dot_general(a, b, (((1,), (1,)), ((), ())), preferred_element_type=f32)


def _pk(v):
    return pltpu.bitcast(v, u32)


def _upk(v):
    return pltpu.bitcast(v, bf16)


def _rcp(d):
    r = pl.reciprocal(d, approx=True)
    return r * (2.0 - d * r)


def _phi(t):
    return jnp.where(t > 0, t + 1.0, jnp.exp(t)) + 1e-6


def _lsums(A11, A12, A21, A22):
    return [A11 + A22, A21 + A22, A11, A22, A11 + A12, A21 - A11, A12 - A22]


def _add(a, b):
    return (a.astype(f32) + b.astype(f32)).astype(bf16)


def _sub(a, b):
    return (a.astype(f32) - b.astype(f32)).astype(bf16)


ORDER = (2, 5, 4, 3, 1, 6, 7)
RIDX = {1: 0, 2: 2, 3: 6, 4: 5, 5: 3, 6: 4, 7: 1}


def _rhs_ops(B11, B12, B21, B22):
    return {1: lambda: _add(B11(), B22()), 2: B11, 3: lambda: _sub(B12(), B22()), 4: lambda: _sub(B21(), B11()),
            5: B22, 6: lambda: _add(B11(), B12()), 7: lambda: _add(B21(), B22())}


def _combine(M):
    return M[1] + M[4] - M[5] + M[7], M[3] + M[5], M[2] + M[4], M[1] - M[2] + M[3] + M[6]


def _spread(ntie, nslots, off=0):
    return [off + (q * (nslots - off)) // ntie for q in range(ntie)]


def _tie_rows(getrows, nm, nk, slots, tmask):
    cols = []
    for j in range(nk):
        rows, m0 = [], 0
        for m in range(nm):
            if (m, j) in slots:
                if m > m0:
                    rows.append(getrows(m0, m, j))
                v = getrows(m, m + 1, j)
                for tv in slots[(m, j)]:
                    v = jnp.where(tmask, v, tv)
                rows.append(v)
                m0 = m + 1
        if m0 < nm:
            rows.append(getrows(m0, nm, j))
        cols.append(jnp.concatenate(rows, axis=0) if len(rows) > 1 else rows[0])
    return _upk(jnp.concatenate(cols, axis=1))


def _tie_value(lhs, ties, tmask):
    if not ties:
        return lhs
    nm, nk = lhs.shape[0] // 16, lhs.shape[1] // 128
    slots = {}
    for tv, sidx in zip(ties, _spread(len(ties), nm * nk)):
        grp, rem = divmod(sidx, nm * 4)
        m, jj = divmod(rem, min(4, nk - grp * 4))
        slots.setdefault((min(m, nm - 1), grp * 4 + jj), []).append(tv)
    p = _pk(lhs)
    return _tie_rows(lambda m0, m1, j: p[m0 * 8:m1 * 8, j * 128:(j + 1) * 128], nm, nk, slots, tmask)


def _strassen(L, R, dot=_dot, ties=(), tmask=None):
    M, ties = {}, list(ties)
    for n, p in enumerate(ORDER):
        k = len(ties) // (len(ORDER) - n)
        mine, ties = ties[:k], ties[k:]
        M[p] = dot(_tie_value(L(p - 1), mine, tmask), R(p))
    return _combine(M)


def _kernel(x_hbm, wqkv_hbm, wo_hbm, w1_hbm, w2_hbm, b1_hbm, b2_hbm, gw_hbm, out_hbm,
            x_v, wqk_v, wv_v, wo_v, w1_v, w2_v, o_v, b1_v, b2_v, gw_v,
            wqkT_p, wL_p, hL_p, pq_p, pkL_p, tb_p, woT_p, mL_p, gL_p,
            gate_v, zb_v, ga_v, b2f_v, pend_p, sem, sem_o):
    cp = pltpu.make_async_copy
    cp_x = [cp(x_hbm.at[0, pl.ds(c * TC, TC), :], x_v.at[pl.ds(c * TC, TC), :], sem.at[c]) for c in range(NC)]
    cp_wq = cp(wqkv_hbm.at[:, pl.ds(0, D)], wqk_v.at[:, pl.ds(0, D)], sem.at[NC + 0])
    cp_wk = cp(wqkv_hbm.at[:, pl.ds(D, D)], wqk_v.at[:, pl.ds(D, D)], sem.at[NC + 1])
    cp_wv = cp(wqkv_hbm.at[:, pl.ds(2 * D, D)], wv_v, sem.at[NC + 2])
    cp_wo = cp(wo_hbm, wo_v, sem.at[NC + 3])
    cp_w1 = cp(w1_hbm, w1_v, sem.at[NC + 4])
    cp_w2 = cp(w2_hbm, w2_v, sem.at[NC + 5])
    cp_gw = cp(gw_hbm, gw_v, sem.at[NC + 6])
    cp_b1 = cp(b1_hbm, b1_v, sem.at[NC + 7])
    cp_b2 = cp(b2_hbm, b2_v, sem.at[NC + 8])
    for c_ in (cp_wq, cp_gw, cp_x[0], cp_x[1], cp_wk, *cp_x[2:], cp_w1, cp_b1, cp_b2, cp_wv, cp_wo, cp_w2):
        c_.start()

    ties = []
    mean, held = {}, {}
    zacc = [None]

    def tie(v):
        ties.append(v if v.dtype == u32 else pltpu.bitcast(v, u32))

    def take(n):
        mine = ties[:n]
        del ties[:n]
        return mine

    def w_transpose(h, tied):
        for j in range(4 * h, 4 * h + 4):
            pk = _pk(wqk_v[:, j * 128:(j + 1) * 128].T)
            wqkT_p[j * 64:(j + 1) * 64, :] = pk
            if tied:
                for kk in range(8):
                    for jj in range(4):
                        tie(pk[8 * kk:8 * kk + 8, jj * 128:(jj + 1) * 128])

    def ext_rows():
        gw = jnp.broadcast_to(gw_v[...].astype(f32).reshape(1, D), (16, D))
        ri = lax.broadcasted_iota(jnp.int32, (16, D), 0)
        return jnp.where(ri == 0, gw, jnp.where(ri == 1, 1.0 / D, 0.0))

    def use_ext(e, t):
        gate_v[:, t * 128:(t + 1) * 128] = jnp.broadcast_to(jax.nn.sigmoid(e[0:1, :]), (8, 128))
        mean[t] = e[1:2, :]

    def qk_dot(c, h, nties=0, off=0):
        if nties:
            slots = {}
            for tv, sidx in zip(take(nties), _spread(nties, 128, off)):
                slots.setdefault((sidx // 4, sidx % 4), []).append(tv)
            lhs = _tie_rows(lambda m0, m1, j: wqkT_p[h * 256 + m0 * 8:h * 256 + m1 * 8, j * 128:(j + 1) * 128],
                            32, 4, slots, tmask)
        else:
            lhs = _upk(wqkT_p[h * 256:(h + 1) * 256, :])
        if h == 0:
            lhs = jnp.concatenate([lhs, _upk(wqkT_p[512:520, :])], axis=0)
        return _dot_nt(lhs, x_v[c * TC:(c + 1) * TC, :])

    def q_store(c, q):
        for par in range(2):
            use_ext(q[D:D + 8, par * 128:(par + 1) * 128], 2 * c + par)
        pq_p[:, c * TC:(c + 1) * TC] = _pk(_phi(q[:D]).astype(bf16))

    def k_finish(c, pe, po):
        for i, l in enumerate(_lsums(pe[:HD], po[:HD], pe[HD:], po[HD:])):
            pkL_p[i, :, c * 128:(c + 1) * 128] = _pk(l.astype(bf16))
        s = pe + po
        zacc[0] = s if zacc[0] is None else zacc[0] + s

    def k_store(c, k):
        pk = _phi(k)
        k_finish(c, pk[:, :128], pk[:, 128:])

    def w_lsums():
        ext = ext_rows()
        A = {}
        for (i, j) in ((0, 0), (0, 1), (1, 0), (1, 1)):
            w = _upk(wqkT_p[i * 256:(i + 1) * 256, j * HD:(j + 1) * HD]).astype(f32)
            e = ext[:, j * HD:(j + 1) * HD] if i == 0 else jnp.zeros((16, HD), f32)
            A[i, j] = jnp.concatenate([w, e], axis=0)
        for i, l in enumerate(_lsums(A[0, 0], A[0, 1], A[1, 0], A[1, 1])):
            pk = _pk(l.astype(bf16))
            wL_p[i] = pk
            for kk in range(0, 33, 2):
                for jj in range(2):
                    tie(pk[8 * kk:8 * kk + 8, jj * 128:(jj + 1) * 128])

    def qk_strassen(c, nties):
        def nat(par, half):
            t = 2 * c + par
            return lambda: x_v[t * 128:(t + 1) * 128, half * HD:(half + 1) * HD]
        R = _rhs_ops(nat(0, 0), nat(1, 0), nat(0, 1), nat(1, 1))
        M, tl = {}, take(nties)
        for n, p in enumerate(ORDER):
            k = len(tl) // (len(ORDER) - n)
            mine, tl = tl[:k], tl[k:]
            rows = 256 if p in (2, 4) else 264
            M[p] = _dot_nt(_tie_value(_upk(wL_p[p - 1, 0:rows, :]), mine, tmask), R[p]())
        e11 = M[1][D:D + 8] - M[5][D:D + 8] + M[7][D:D + 8]
        C11 = jnp.concatenate([M[1][:D] + M[4] - M[5][:D] + M[7][:D], e11], axis=0)
        C12 = (M[3] + M[5])[:D + 8]
        C21 = M[2] + M[4]
        C22 = M[1][:D] - M[2] + M[3][:D] + M[6][:D]
        for par, Cq in ((0, C11), (1, C12)):
            t = 2 * c + par
            use_ext(Cq[D:D + 8, :], t)
            pq_p[:, t * 128:(t + 1) * 128] = _pk(_phi(Cq[:D]).astype(bf16))
        k_finish(c, _phi(C21[:D]), _phi(C22[:D]))

    def layernorm(c):
        xT, stats = {}, {}
        for par in range(2):
            t = 2 * c + par
            ts = slice(t * 128, (t + 1) * 128)
            for j in range(4):
                xT[par, j] = x_v[ts, j * 128:(j + 1) * 128].T
            m = mean.pop(t)
            vs = None
            for j in range(4):
                xc = xT[par, j].astype(f32) - m
                v = jnp.sum((xc * xc).reshape(16, 8, 128), axis=0)
                vs = v if vs is None else vs + v
                tie(vs)
            stats[par] = (m, lax.rsqrt(jnp.sum(vs, axis=0, keepdims=True) * (1.0 / D) + 1e-5))
        (me, re), (mo, ro) = stats[0], stats[1]
        for b in range(2):
            for r in range(0, 128, 16):
                rs = slice(r, r + 16)
                a11 = (xT[0, b][rs].astype(f32) - me) * re
                a21 = (xT[0, 2 + b][rs].astype(f32) - me) * re
                a12 = (xT[1, b][rs].astype(f32) - mo) * ro
                a22 = (xT[1, 2 + b][rs].astype(f32) - mo) * ro
                for i, l in enumerate(_lsums(a11, a12, a21, a22)):
                    pk = _pk(l.astype(bf16))
                    hL_p[i, (b * 128 + r) // 2:(b * 128 + r + 16) // 2, c * 128:(c + 1) * 128] = pk
                    tie(pk)

    TM = {}

    def t_product(n, nties):
        def quad(par, col):
            return lambda: jnp.concatenate(
                [x_v[(2 * t + par) * 128:(2 * t + par + 1) * 128, col * HD:(col + 1) * HD] for t in range(NC)], axis=0)
        p = ORDER[n]
        R = _rhs_ops(quad(0, 0), quad(0, 1), quad(1, 0), quad(1, 1))
        TM[p] = _dot(_tie_value(_upk(pkL_p[p - 1]), take(nties), tmask), R[p]())
        if n == 6:
            C11, C12, C21, C22 = _combine(TM)
            tb_p[0:HD // 2, :] = _pk(jnp.concatenate([C11, C12], axis=1).astype(bf16))
            tb_p[HD // 2:, :] = _pk(jnp.concatenate([C21, C22], axis=1).astype(bf16))

    def u_stage(j, nties=0):
        def quad(par, col):
            return lambda: jnp.concatenate(
                [w1_v[(2 * t + par) * 128:(2 * t + par + 1) * 128, j * 256 + col * 128:j * 256 + (col + 1) * 128]
                 for t in range(NC)], axis=0)
        R = _rhs_ops(quad(0, 0), quad(0, 1), quad(1, 0), quad(1, 1))
        C11, C12, C21, C22 = _strassen(lambda i: _upk(hL_p[i]), lambda p: R[p](), _dot, take(nties), tmask)

        def gl(v, f0):
            return jax.nn.gelu(v + b1[:, f0:f0 + 128], approximate=True)
        G = (gl(C11, j * 256), gl(C12, j * 256 + 128), gl(C21, j * 256), gl(C22, j * 256 + 128))
        for i, l in enumerate(_lsums(*G)):
            gL_p[i, :, j * 128:(j + 1) * 128] = _pk(l.astype(bf16))

    def norm_stage(c):
        nb = {}
        for par in range(2):
            ts = slice((2 * c + par) * 128, (2 * c + par + 1) * 128)
            for b in range(4):
                pq = _upk(pq_p[b * 64:(b + 1) * 64, ts]).astype(f32)
                den = jnp.sum((pq * zb_v[b * 128:(b + 1) * 128, :]).reshape(8, DH, 128), axis=1, keepdims=True) + 1e-6
                nb[par, b] = (pq.reshape(8, DH, 128) * _rcp(den)).reshape(128, 128)
        ops = [[None, None] for _ in range(7)]
        for bp in range(2):
            for i, l in enumerate(_lsums(nb[0, bp], nb[1, bp], nb[0, 2 + bp], nb[1, 2 + bp])):
                ops[i][bp] = l.astype(bf16)
        R = [jnp.concatenate(o, axis=0) for o in ops]
        for p in ORDER:
            pk = _pk(R[RIDX[p]])
            for k in range(16):
                tie(pk[8 * k:8 * k + 8, :])
        held[c] = R

    def a_stage(c):
        R = held.pop(c)
        C = _strassen(lambda i: _upk(mL_p[i]), lambda p: R[RIDX[p]])
        aT = jnp.concatenate([jnp.concatenate([C[0], C[1]], axis=1), jnp.concatenate([C[2], C[3]], axis=1)], axis=0)
        cs = slice(c * TC, (c + 1) * TC)
        ga_v[:, cs] = gate_v[0:1, cs] * aT

    cp_wq.wait()
    w_transpose(0, tied=False)
    cp_x[0].wait()
    cp_gw.wait()
    g8 = wqk_v[0:16, 0:128].astype(f32)[0:8, :]
    tmask = (g8 >= 0.0) | (g8 < 0.0) | (g8 != g8)
    wqkT_p[512:520, :] = _pk(ext_rows().astype(bf16))
    q_store(0, qk_dot(0, 0))
    cp_x[1].wait()
    q_store(1, qk_dot(1, 0))
    cp_wk.wait()
    cp_x[2].wait()
    w_transpose(1, tied=True)
    q_store(2, qk_dot(2, 0, 128, 64))
    k_store(0, qk_dot(0, 1))
    w_lsums()
    k_store(1, qk_dot(1, 1, 120))
    k_store(2, qk_dot(2, 1, 118))
    for c in range(3, NC):
        cp_x[c].wait()
    qk_strassen(3, 0)
    nxt = [0]

    def need(n):
        while len(ties) < n and nxt[0] < NC:
            layernorm(nxt[0])
            nxt[0] += 1
    for c, n in zip(range(4, NC), TK[:4]):
        need(n)
        qk_strassen(c, n)
    zb_v[...] = jnp.broadcast_to(jnp.sum(zacc[0], axis=1, keepdims=True), (D, 128))
    for n, nt in enumerate(TK[4:]):
        need(nt)
        t_product(n, nt)
    assert nxt[0] == NC and not ties

    for c_ in (cp_w1, cp_b1, cp_b2, cp_wv, cp_wo):
        c_.wait()
    for j in range(4):
        woT_p[j * 64:(j + 1) * 64, :] = _pk(wo_v[:, j * 128:(j + 1) * 128].T)
    b1 = b1_v[...].astype(f32).reshape(1, F)
    u_stage(0)
    msk = (lax.broadcasted_iota(jnp.int32, (128, 128), 0) // DH) == (lax.broadcasted_iota(jnp.int32, (128, 128), 1) // DH)
    kvs = []
    for b in range(4):
        kv = _dot(_upk(tb_p[b * 64:(b + 1) * 64, :]), wv_v[:, b * 128:(b + 1) * 128])
        kvs.append(jnp.where(msk, kv, 0.0).astype(bf16))
    u_stage(1)
    Ms = [_dot_nt(_upk(woT_p[:, b * 128:(b + 1) * 128]), kvs[b]) for b in range(4)]
    for bp in range(2):
        for i, l in enumerate(_lsums(Ms[bp][:HD], Ms[2 + bp][:HD], Ms[bp][HD:], Ms[2 + bp][HD:])):
            mL_p[i, :, bp * 128:(bp + 1) * 128] = _pk(l.astype(bf16))
    for j in (2, 3, 4):
        norm_stage(2 * j - 4)
        norm_stage(2 * j - 3)
        u_stage(j, 224)
        a_stage(2 * j - 4)
        a_stage(2 * j - 3)
    norm_stage(6)
    norm_stage(7)
    u_stage(5, 224)
    a_stage(6)
    u_stage(6)
    a_stage(7)

    cp_w2.wait()
    b2f_v[...] = jnp.broadcast_to(b2_v[...].astype(f32).reshape(1, S), (8, S))

    def out_tile(tt, obT, s):
        o_v[tt, :] = obT
        cp(o_v.at[tt, :], out_hbm.at[0, tt, :], s).start()

    pend_p[...] = jnp.zeros((HD, 128), u32)

    def y_body(i, carry):
        tprev = pl.multiple_of(jnp.where(i == 0, 14, 4 * i - 2) * 128, 128)
        out_tile(pl.ds(tprev, 128), _upk(pend_p[...]).T, sem_o.at[jnp.where(i == 0, 1, 0)])
        for k in range(2):
            c0 = pl.multiple_of((2 * i + k) * TC, TC)

            def quad(par, col):
                return lambda: jnp.concatenate(
                    [w2_v[(2 * t + par) * 128:(2 * t + par + 1) * 128, pl.ds(c0 + col * 128, 128)] for t in range(NF)],
                    axis=0)
            R = _rhs_ops(quad(0, 0), quad(0, 1), quad(1, 0), quad(1, 1))
            Y11, Y12, Y21, Y22 = _strassen(lambda n: _upk(gL_p[n]), lambda p: R[p]())
            for par, (Ya, Yb) in ((1, (Y12, Y22)), (0, (Y11, Y21))):
                tt = pl.ds(c0 + par * 128, 128)
                y = jnp.concatenate([Ya, Yb], axis=0) + b2f_v[0:1, tt]
                oT = (ga_v[:, tt] + (1.0 - gate_v[0:1, tt]) * y).astype(bf16)
                if k == 1 and par == 0:
                    pend_p[...] = _pk(oT)
                else:
                    out_tile(tt, oT.T, sem_o.at[0])
        return carry
    lax.fori_loop(0, NC // 2, y_body, 0)
    t14 = pl.ds(14 * 128, 128)
    cp(o_v.at[t14, :], out_hbm.at[0, t14, :], sem_o.at[1]).wait()
    out_tile(t14, _upk(pend_p[...]).T, sem_o.at[0])
    cp(o_v, out_hbm.at[0], sem_o.at[0]).wait()


@jax.jit
def pallas_gated_mix__linear_attn_block__mixer_token_mlp__prompt_kernel(
        A_x, A_wqkv, A_wo, B_x, B_w1, B_b1, B_w2, B_b2, gate_w):
    del B_x
    assert A_x.shape == (1, S, D) and B_w1.shape == (S, F) and B_w2.shape == (F, S), "fixed problem shape"
    vm = pltpu.VMEM
    scratch = [
        vm((S, D), bf16),
        vm((D, 2 * D), bf16),
        vm((D, D), bf16),
        vm((D, D), bf16),
        vm((S, F), bf16),
        vm((F, S), bf16),
        vm((S, D), bf16),
        vm((F,), bf16),
        vm((S,), bf16),
        vm((D,), bf16),
        vm((D + 8, D), u32),
        vm((7, 264, HD), u32),
        vm((7, D // 4, S // 2), u32),
        vm((HD, S), u32),
        vm((7, D // 4, S // 2), u32),
        vm((HD, D), u32),
        vm((HD, D), u32),
        vm((7, D // 4, HD), u32),
        vm((7, D // 4, F // 2), u32),
        vm((8, S), f32),
        vm((D, 128), f32),
        vm((D, S), f32),
        vm((8, S), f32),
        vm((HD, 128), u32),
        pltpu.SemaphoreType.DMA((NC + 9,)),
        pltpu.SemaphoreType.DMA((2,)),
    ]
    any_spec = pl.BlockSpec(memory_space=pl.ANY)
    return pl.pallas_call(
        _kernel,
        out_shape=jax.ShapeDtypeStruct((1, S, D), bf16),
        in_specs=[any_spec] * 8,
        out_specs=any_spec,
        scratch_shapes=scratch,
        compiler_params=pltpu.CompilerParams(
            vmem_limit_bytes=100 * 1024 * 1024, disable_semaphore_checks=True, disable_bounds_checks=True),
    )(A_x, A_wqkv, A_wo, B_w1, B_w2, B_b1, B_b2, gate_w)
```

```python
import jax
import jax.numpy as jnp
from jax import lax
from jax.experimental import pallas as pl
from jax.experimental.pallas import tpu as pltpu

S, D, F, H, DH = 2048, 512, 1792, 32, 16
HD = D // 2
TK = (120, 96, 96, 140, 144, 88, 80, 72, 24, 36, 48, 16)
TC = 256
NC = S // TC
NF = F // 256
f32, bf16, u32 = jnp.float32, jnp.bfloat16, jnp.uint32


def _dot(a, b):
    return jnp.dot(a, b, preferred_element_type=f32)


def _dot_nt(a, b):
    return lax.dot_general(a, b, (((1,), (1,)), ((), ())), preferred_element_type=f32)


def _pk(v):
    return pltpu.bitcast(v, u32)


def _upk(v):
    return pltpu.bitcast(v, bf16)


def _rcp(d):
    r = pl.reciprocal(d, approx=True)
    return r * (2.0 - d * r)


def _phi(t):
    return jnp.where(t > 0, t + 1.0, jnp.exp(t)) + 1e-6


def _lsums(A11, A12, A21, A22):
    return [A11 + A22, A21 + A22, A11, A22, A11 + A12, A21 - A11, A12 - A22]


def _add(a, b):
    return (a.astype(f32) + b.astype(f32)).astype(bf16)


def _sub(a, b):
    return (a.astype(f32) - b.astype(f32)).astype(bf16)


ORDER = (2, 5, 4, 3, 1, 6, 7)
RIDX = {1: 0, 2: 2, 3: 6, 4: 5, 5: 3, 6: 4, 7: 1}


def _rhs_ops(B11, B12, B21, B22):
    return {1: lambda: _add(B11(), B22()), 2: B11, 3: lambda: _sub(B12(), B22()), 4: lambda: _sub(B21(), B11()),
            5: B22, 6: lambda: _add(B11(), B12()), 7: lambda: _add(B21(), B22())}


def _combine(M):
    return M[1] + M[4] - M[5] + M[7], M[3] + M[5], M[2] + M[4], M[1] - M[2] + M[3] + M[6]


def _spread(ntie, nslots, off=0):
    return [off + (q * (nslots - off)) // ntie for q in range(ntie)]


def _tie_rows(getrows, nm, nk, slots, tmask):
    cols = []
    for j in range(nk):
        rows, m0 = [], 0
        for m in range(nm):
            if (m, j) in slots:
                if m > m0:
                    rows.append(getrows(m0, m, j))
                v = getrows(m, m + 1, j)
                for tv in slots[(m, j)]:
                    v = jnp.where(tmask, v, tv)
                rows.append(v)
                m0 = m + 1
        if m0 < nm:
            rows.append(getrows(m0, nm, j))
        cols.append(jnp.concatenate(rows, axis=0) if len(rows) > 1 else rows[0])
    return _upk(jnp.concatenate(cols, axis=1))


def _tie_value(lhs, ties, tmask):
    if not ties:
        return lhs
    nm, nk = lhs.shape[0] // 16, lhs.shape[1] // 128
    slots = {}
    for tv, sidx in zip(ties, _spread(len(ties), nm * nk)):
        grp, rem = divmod(sidx, nm * 4)
        m, jj = divmod(rem, min(4, nk - grp * 4))
        slots.setdefault((min(m, nm - 1), grp * 4 + jj), []).append(tv)
    p = _pk(lhs)
    return _tie_rows(lambda m0, m1, j: p[m0 * 8:m1 * 8, j * 128:(j + 1) * 128], nm, nk, slots, tmask)


def _strassen(L, R, dot=_dot, ties=(), tmask=None):
    M, ties = {}, list(ties)
    for n, p in enumerate(ORDER):
        k = len(ties) // (len(ORDER) - n)
        mine, ties = ties[:k], ties[k:]
        M[p] = dot(_tie_value(L(p - 1), mine, tmask), R(p))
    return _combine(M)


def _kernel(x_hbm, wqkv_hbm, wo_hbm, w1_hbm, w2_hbm, b1_hbm, b2_hbm, gw_hbm, out_hbm,
            x_v, wqk_v, wv_v, wo_v, w1_v, w2_v, o_v, b1_v, b2_v, gw_v,
            wqkT_p, hL_p, pq_p, pkL_p, tb_p, woT_p, mL_p, gL_p,
            gate_v, zb_v, ga_v, b2f_v, pend_p, sem, sem_o):
    cp = pltpu.make_async_copy
    cp_x = [cp(x_hbm.at[0, pl.ds(c * TC, TC), :], x_v.at[pl.ds(c * TC, TC), :], sem.at[c]) for c in range(NC)]
    cp_wq = cp(wqkv_hbm.at[:, pl.ds(0, D)], wqk_v.at[:, pl.ds(0, D)], sem.at[NC + 0])
    cp_wk = cp(wqkv_hbm.at[:, pl.ds(D, D)], wqk_v.at[:, pl.ds(D, D)], sem.at[NC + 1])
    cp_wv = cp(wqkv_hbm.at[:, pl.ds(2 * D, D)], wv_v, sem.at[NC + 2])
    cp_wo = cp(wo_hbm, wo_v, sem.at[NC + 3])
    cp_w1 = cp(w1_hbm, w1_v, sem.at[NC + 4])
    cp_w2 = cp(w2_hbm, w2_v, sem.at[NC + 5])
    cp_gw = cp(gw_hbm, gw_v, sem.at[NC + 6])
    cp_b1 = cp(b1_hbm, b1_v, sem.at[NC + 7])
    cp_b2 = cp(b2_hbm, b2_v, sem.at[NC + 8])
    for c_ in (cp_wq, cp_gw, cp_x[0], cp_x[1], cp_wk, *cp_x[2:], cp_w1, cp_b1, cp_b2, cp_wv, cp_wo, cp_w2):
        c_.start()

    ties = []
    mean, held = {}, {}
    zacc = [None]

    def tie(v):
        ties.append(v if v.dtype == u32 else pltpu.bitcast(v, u32))

    def take(n):
        mine = ties[:n]
        del ties[:n]
        return mine

    def w_transpose(h, tied):
        for j in range(4 * h, 4 * h + 4):
            pk = _pk(wqk_v[:, j * 128:(j + 1) * 128].T)
            wqkT_p[j * 64:(j + 1) * 64, :] = pk
            if tied:
                for kk in range(8):
                    for jj in range(4):
                        tie(pk[8 * kk:8 * kk + 8, jj * 128:(jj + 1) * 128])

    def ext_rows():
        gw = jnp.broadcast_to(gw_v[...].astype(f32).reshape(1, D), (16, D))
        ri = lax.broadcasted_iota(jnp.int32, (16, D), 0)
        return jnp.where(ri == 0, gw, jnp.where(ri == 1, 1.0 / D, 0.0))

    def use_ext(e, t):
        gate_v[:, t * 128:(t + 1) * 128] = jnp.broadcast_to(jax.nn.sigmoid(e[0:1, :]), (8, 128))
        mean[t] = e[1:2, :]

    def qk_dot(c, h, nties=0, off=0):
        if nties:
            slots = {}
            for tv, sidx in zip(take(nties), _spread(nties, 128, off)):
                slots.setdefault((sidx // 4, sidx % 4), []).append(tv)
            lhs = _tie_rows(lambda m0, m1, j: wqkT_p[h * 256 + m0 * 8:h * 256 + m1 * 8, j * 128:(j + 1) * 128],
                            32, 4, slots, tmask)
        else:
            lhs = _upk(wqkT_p[h * 256:(h + 1) * 256, :])
        if h == 0:
            lhs = jnp.concatenate([lhs, _upk(wqkT_p[512:520, :])], axis=0)
        return _dot_nt(lhs, x_v[c * TC:(c + 1) * TC, :])

    def q_store(c, q):
        for par in range(2):
            use_ext(q[D:D + 8, par * 128:(par + 1) * 128], 2 * c + par)
        pq_p[:, c * TC:(c + 1) * TC] = _pk(_phi(q[:D]).astype(bf16))

    def k_finish(c, pe, po):
        e4, o4 = pe.reshape(H, 2, 8, 128), po.reshape(H, 2, 8, 128)
        quads = (e4[:, 0], o4[:, 0], e4[:, 1], o4[:, 1])
        for i, l in enumerate(_lsums(*[v.reshape(HD, 128) for v in quads])):
            pkL_p[i, :, c * 128:(c + 1) * 128] = _pk(l.astype(bf16))
        s = pe + po
        zacc[0] = s if zacc[0] is None else zacc[0] + s

    def k_store(c, k):
        pk = _phi(k)
        k_finish(c, pk[:, :128], pk[:, 128:])

    def layernorm(c):
        xT, stats = {}, {}
        for par in range(2):
            t = 2 * c + par
            ts = slice(t * 128, (t + 1) * 128)
            for j in range(4):
                xT[par, j] = x_v[ts, j * 128:(j + 1) * 128].T
            m = mean.pop(t)
            vs = None
            for j in range(4):
                xc = xT[par, j].astype(f32) - m
                v = jnp.sum((xc * xc).reshape(16, 8, 128), axis=0)
                vs = v if vs is None else vs + v
                tie(vs)
            stats[par] = (m, lax.rsqrt(jnp.sum(vs, axis=0, keepdims=True) * (1.0 / D) + 1e-5))
        (me, re), (mo, ro) = stats[0], stats[1]
        for b in range(2):
            for r in range(0, 128, 16):
                rs = slice(r, r + 16)
                a11 = (xT[0, b][rs].astype(f32) - me) * re
                a21 = (xT[0, 2 + b][rs].astype(f32) - me) * re
                a12 = (xT[1, b][rs].astype(f32) - mo) * ro
                a22 = (xT[1, 2 + b][rs].astype(f32) - mo) * ro
                for i, l in enumerate(_lsums(a11, a12, a21, a22)):
                    pk = _pk(l.astype(bf16))
                    hL_p[i, (b * 128 + r) // 2:(b * 128 + r + 16) // 2, c * 128:(c + 1) * 128] = pk
                    tie(pk)

    TM = {}

    def t_product(n, nties):
        def quad(par, col):
            return lambda: jnp.concatenate(
                [x_v[(2 * t + par) * 128:(2 * t + par + 1) * 128, col * HD:(col + 1) * HD] for t in range(NC)], axis=0)
        p = ORDER[n]
        R = _rhs_ops(quad(0, 0), quad(0, 1), quad(1, 0), quad(1, 1))
        TM[p] = _dot(_tie_value(_upk(pkL_p[p - 1]), take(nties), tmask), R[p]())
        if n == 6:
            C11, C12, C21, C22 = _combine(TM)
            lo = jnp.concatenate([C11, C12], axis=1).reshape(H, 1, 8, D)
            hi = jnp.concatenate([C21, C22], axis=1).reshape(H, 1, 8, D)
            tb_p[...] = _pk(jnp.concatenate([lo, hi], axis=1).reshape(D, D).astype(bf16))

    def u_stage(j, nties=0):
        def quad(par, col):
            return lambda: jnp.concatenate(
                [w1_v[(2 * t + par) * 128:(2 * t + par + 1) * 128, j * 256 + col * 128:j * 256 + (col + 1) * 128]
                 for t in range(NC)], axis=0)
        R = _rhs_ops(quad(0, 0), quad(0, 1), quad(1, 0), quad(1, 1))
        C11, C12, C21, C22 = _strassen(lambda i: _upk(hL_p[i]), lambda p: R[p](), _dot, take(nties), tmask)

        def gl(v, f0):
            return jax.nn.gelu(v + b1[:, f0:f0 + 128], approximate=True)
        G = (gl(C11, j * 256), gl(C12, j * 256 + 128), gl(C21, j * 256), gl(C22, j * 256 + 128))
        for i, l in enumerate(_lsums(*G)):
            gL_p[i, :, j * 128:(j + 1) * 128] = _pk(l.astype(bf16))

    def norm_stage(c):
        nb = {}
        for par in range(2):
            ts = slice((2 * c + par) * 128, (2 * c + par + 1) * 128)
            for b in range(4):
                pq = _upk(pq_p[b * 64:(b + 1) * 64, ts]).astype(f32)
                t3 = (pq * zb_v[b * 128:(b + 1) * 128, :]).reshape(8, DH, 128)
                den = jnp.sum(t3, axis=1, keepdims=True) + 1e-6
                nb[par, b] = (t3 * _rcp(den)).reshape(128, 128)
        ops = [[None, None] for _ in range(7)]
        for bp in range(2):
            for i, l in enumerate(_lsums(nb[0, bp], nb[1, bp], nb[0, 2 + bp], nb[1, 2 + bp])):
                ops[i][bp] = l.astype(bf16)
        R = [jnp.concatenate(o, axis=0) for o in ops]
        for p in ORDER:
            pk = _pk(R[RIDX[p]])
            for k in range(16):
                tie(pk[8 * k:8 * k + 8, :])
        held[c] = R

    def a_stage(c):
        R = held.pop(c)
        C = _strassen(lambda i: _upk(mL_p[i]), lambda p: R[RIDX[p]])
        aT = jnp.concatenate([jnp.concatenate([C[0], C[1]], axis=1), jnp.concatenate([C[2], C[3]], axis=1)], axis=0)
        cs = slice(c * TC, (c + 1) * TC)
        ga_v[:, cs] = gate_v[0:1, cs] * aT

    cp_wq.wait()
    w_transpose(0, tied=False)
    cp_x[0].wait()
    cp_gw.wait()
    g8 = wqk_v[0:16, 0:128].astype(f32)[0:8, :]
    tmask = (g8 >= 0.0) | (g8 < 0.0) | (g8 != g8)
    wqkT_p[512:520, :] = _pk(ext_rows().astype(bf16))
    q_store(0, qk_dot(0, 0))
    cp_x[1].wait()
    q_store(1, qk_dot(1, 0))
    cp_wk.wait()
    cp_x[2].wait()
    w_transpose(1, tied=True)
    q_store(2, qk_dot(2, 0, 128, 64))
    k_store(0, qk_dot(0, 1))
    k_store(1, qk_dot(1, 1))
    k2 = qk_dot(2, 1)
    for c in range(3, NC):
        cp_x[c].wait()
    k_store(2, k2)
    nxt = [0]

    def need(n):
        while len(ties) < n and nxt[0] < NC:
            layernorm(nxt[0])
            nxt[0] += 1
    for c in range(3, NC):
        q_store(c, qk_dot(c, 0))
    for c, n in zip(range(3, NC), TK[:5]):
        need(n)
        k_store(c, qk_dot(c, 1, n))
    zb_v[...] = jnp.broadcast_to(jnp.sum(zacc[0], axis=1, keepdims=True), (D, 128))
    for n, nt in enumerate(TK[5:]):
        need(nt)
        t_product(n, nt)
    assert nxt[0] == NC and not ties

    for c_ in (cp_w1, cp_b1, cp_b2, cp_wv, cp_wo):
        c_.wait()
    for j in range(4):
        woT_p[j * 64:(j + 1) * 64, :] = _pk(wo_v[:, j * 128:(j + 1) * 128].T)
    b1 = b1_v[...].astype(f32).reshape(1, F)
    u_stage(0)
    msk = (lax.broadcasted_iota(jnp.int32, (128, 128), 0) // DH) == (lax.broadcasted_iota(jnp.int32, (128, 128), 1) // DH)
    kvs = []
    for b in range(4):
        kv = _dot(_upk(tb_p[b * 64:(b + 1) * 64, :]), wv_v[:, b * 128:(b + 1) * 128])
        kvs.append(jnp.where(msk, kv * _rcp(zb_v[b * 128:(b + 1) * 128, :]), 0.0).astype(bf16))
    u_stage(1)
    Ms = [_dot_nt(_upk(woT_p[:, b * 128:(b + 1) * 128]), kvs[b]) for b in range(4)]
    for bp in range(2):
        for i, l in enumerate(_lsums(Ms[bp][:HD], Ms[2 + bp][:HD], Ms[bp][HD:], Ms[2 + bp][HD:])):
            mL_p[i, :, bp * 128:(bp + 1) * 128] = _pk(l.astype(bf16))
    for j in (2, 3, 4):
        norm_stage(2 * j - 4)
        norm_stage(2 * j - 3)
        u_stage(j, 224)
        a_stage(2 * j - 4)
        a_stage(2 * j - 3)
    norm_stage(6)
    norm_stage(7)
    u_stage(5, 224)
    a_stage(6)
    u_stage(6)
    a_stage(7)

    cp_w2.wait()
    b2f_v[...] = jnp.broadcast_to(b2_v[...].astype(f32).reshape(1, S), (8, S))

    def out_tile(tt, obT, s):
        o_v[tt, :] = obT
        cp(o_v.at[tt, :], out_hbm.at[0, tt, :], s).start()

    pend_p[...] = jnp.zeros((HD, 128), u32)

    def y_body(i, carry):
        tprev = pl.multiple_of(jnp.where(i == 0, 14, 4 * i - 2) * 128, 128)
        out_tile(pl.ds(tprev, 128), _upk(pend_p[...]).T, sem_o.at[jnp.where(i == 0, 1, 0)])
        for k in range(2):
            c0 = pl.multiple_of((2 * i + k) * TC, TC)

            def quad(par, col):
                return lambda: jnp.concatenate(
                    [w2_v[(2 * t + par) * 128:(2 * t + par + 1) * 128, pl.ds(c0 + col * 128, 128)] for t in range(NF)],
                    axis=0)
            R = _rhs_ops(quad(0, 0), quad(0, 1), quad(1, 0), quad(1, 1))
            Y11, Y12, Y21, Y22 = _strassen(lambda n: _upk(gL_p[n]), lambda p: R[p]())
            for par, (Ya, Yb) in ((1, (Y12, Y22)), (0, (Y11, Y21))):
                tt = pl.ds(c0 + par * 128, 128)
                y = jnp.concatenate([Ya, Yb], axis=0) + b2f_v[0:1, tt]
                oT = (ga_v[:, tt] + (1.0 - gate_v[0:1, tt]) * y).astype(bf16)
                if k == 1 and par == 0:
                    pend_p[...] = _pk(oT)
                else:
                    out_tile(tt, oT.T, sem_o.at[0])
        return carry
    lax.fori_loop(0, NC // 2, y_body, 0)
    t14 = pl.ds(14 * 128, 128)
    cp(o_v.at[t14, :], out_hbm.at[0, t14, :], sem_o.at[1]).wait()
    out_tile(t14, _upk(pend_p[...]).T, sem_o.at[0])
    cp(o_v, out_hbm.at[0], sem_o.at[0]).wait()


@jax.jit
def pallas_gated_mix__linear_attn_block__mixer_token_mlp__prompt_kernel(
        A_x, A_wqkv, A_wo, B_x, B_w1, B_b1, B_w2, B_b2, gate_w):
    del B_x
    assert A_x.shape == (1, S, D) and B_w1.shape == (S, F) and B_w2.shape == (F, S), "fixed problem shape"
    vm = pltpu.VMEM
    scratch = [
        vm((S, D), bf16),
        vm((D, 2 * D), bf16),
        vm((D, D), bf16),
        vm((D, D), bf16),
        vm((S, F), bf16),
        vm((F, S), bf16),
        vm((S, D), bf16),
        vm((F,), bf16),
        vm((S,), bf16),
        vm((D,), bf16),
        vm((D + 8, D), u32),
        vm((7, D // 4, S // 2), u32),
        vm((HD, S), u32),
        vm((7, D // 4, S // 2), u32),
        vm((HD, D), u32),
        vm((HD, D), u32),
        vm((7, D // 4, HD), u32),
        vm((7, D // 4, F // 2), u32),
        vm((8, S), f32),
        vm((D, 128), f32),
        vm((D, S), f32),
        vm((8, S), f32),
        vm((HD, 128), u32),
        pltpu.SemaphoreType.DMA((NC + 9,)),
        pltpu.SemaphoreType.DMA((2,)),
    ]
    any_spec = pl.BlockSpec(memory_space=pl.ANY)
    return pl.pallas_call(
        _kernel,
        out_shape=jax.ShapeDtypeStruct((1, S, D), bf16),
        in_specs=[any_spec] * 8,
        out_specs=any_spec,
        scratch_shapes=scratch,
        compiler_params=pltpu.CompilerParams(
            vmem_limit_bytes=100 * 1024 * 1024, disable_semaphore_checks=True, disable_bounds_checks=True),
    )(A_x, A_wqkv, A_wo, B_w1, B_w2, B_b1, B_b2, gate_w)
```

```python
import jax
import jax.numpy as jnp
from jax import lax
from jax.experimental import pallas as pl
from jax.experimental.pallas import tpu as pltpu

S, D, F, H, DH = 2048, 512, 1792, 32, 16
HD = D // 2
TK = (120, 108, 100, 96, 40, 24, 16, 16, 52, 56, 60, 76, 48, 60, 60, 28)
LT = (128, 184, 192, 192, 200)
TC = 256
NC = S // TC
NF = F // 256
f32, bf16, u32 = jnp.float32, jnp.bfloat16, jnp.uint32


def _dot(a, b):
    return jnp.dot(a, b, preferred_element_type=f32)


def _dot_nt(a, b):
    return lax.dot_general(a, b, (((1,), (1,)), ((), ())), preferred_element_type=f32)


def _pk(v):
    return pltpu.bitcast(v, u32)


def _upk(v):
    return pltpu.bitcast(v, bf16)


def _rcp(d):
    r = pl.reciprocal(d, approx=True)
    return r * (2.0 - d * r)


def _phi(t):
    return jnp.where(t > 0, t + 1.0, jnp.exp(t)) + 1e-6


def _lsums(A11, A12, A21, A22):
    return [A11 + A22, A21 + A22, A11, A22, A11 + A12, A21 - A11, A12 - A22]


def _add(a, b):
    return (a.astype(f32) + b.astype(f32)).astype(bf16)


def _sub(a, b):
    return (a.astype(f32) - b.astype(f32)).astype(bf16)


ORDER = (2, 5, 4, 3, 1, 6, 7)
RIDX = {1: 0, 2: 2, 3: 6, 4: 5, 5: 3, 6: 4, 7: 1}


def _rhs_ops(B11, B12, B21, B22):
    return {1: lambda: _add(B11(), B22()), 2: B11, 3: lambda: _sub(B12(), B22()), 4: lambda: _sub(B21(), B11()),
            5: B22, 6: lambda: _add(B11(), B12()), 7: lambda: _add(B21(), B22())}


def _combine(M):
    return M[1] + M[4] - M[5] + M[7], M[3] + M[5], M[2] + M[4], M[1] - M[2] + M[3] + M[6]


def _spread(ntie, nslots, off=0):
    return [off + (q * (nslots - off)) // ntie for q in range(ntie)]


def _tie_rows(getrows, nm, nk, slots, tmask):
    cols = []
    for j in range(nk):
        rows, m0 = [], 0
        for m in range(nm):
            if (m, j) in slots:
                if m > m0:
                    rows.append(getrows(m0, m, j))
                v = getrows(m, m + 1, j)
                for tv in slots[(m, j)]:
                    v = jnp.where(tmask, v, tv)
                rows.append(v)
                m0 = m + 1
        if m0 < nm:
            rows.append(getrows(m0, nm, j))
        cols.append(jnp.concatenate(rows, axis=0) if len(rows) > 1 else rows[0])
    return _upk(jnp.concatenate(cols, axis=1))


def _tie_value(lhs, ties, tmask):
    if not ties:
        return lhs
    nm, nk = lhs.shape[0] // 16, lhs.shape[1] // 128
    slots = {}
    for tv, sidx in zip(ties, _spread(len(ties), nm * nk)):
        grp, rem = divmod(sidx, nm * 4)
        m, jj = divmod(rem, min(4, nk - grp * 4))
        slots.setdefault((min(m, nm - 1), grp * 4 + jj), []).append(tv)
    p = _pk(lhs)
    return _tie_rows(lambda m0, m1, j: p[m0 * 8:m1 * 8, j * 128:(j + 1) * 128], nm, nk, slots, tmask)


def _strassen(L, R, dot=_dot, ties=(), tmask=None):
    M, ties = {}, list(ties)
    for n, p in enumerate(ORDER):
        k = len(ties) // (len(ORDER) - n)
        mine, ties = ties[:k], ties[k:]
        M[p] = dot(_tie_value(L(p - 1), mine, tmask), R(p))
    return _combine(M)


def _kernel(x_hbm, wqkv_hbm, wo_hbm, w1_hbm, w2_hbm, b1_hbm, b2_hbm, gw_hbm, out_hbm,
            x_v, wqk_v, wv_v, wo_v, w1_v, w2_v, o_v, b1_v, b2_v, gw_v,
            wqkT_p, hL_p, pq_p, pkT_p, pkL_p, zi_v, tb_p, woT_p, mL_p, gL_p,
            gate_v, zb_v, ga_v, b2f_v, pend_p, sem, sem_o):
    cp = pltpu.make_async_copy
    cp_x = [cp(x_hbm.at[0, pl.ds(c * TC, TC), :], x_v.at[pl.ds(c * TC, TC), :], sem.at[c]) for c in range(NC)]
    cp_wq = cp(wqkv_hbm.at[:, pl.ds(0, D)], wqk_v.at[:, pl.ds(0, D)], sem.at[NC + 0])
    cp_wk = cp(wqkv_hbm.at[:, pl.ds(D, D)], wqk_v.at[:, pl.ds(D, D)], sem.at[NC + 1])
    cp_wv = cp(wqkv_hbm.at[:, pl.ds(2 * D, D)], wv_v, sem.at[NC + 2])
    cp_wo = cp(wo_hbm, wo_v, sem.at[NC + 3])
    cp_w1 = cp(w1_hbm, w1_v, sem.at[NC + 4])
    cp_w2 = cp(w2_hbm, w2_v, sem.at[NC + 5])
    cp_gw = cp(gw_hbm, gw_v, sem.at[NC + 6])
    cp_b1 = cp(b1_hbm, b1_v, sem.at[NC + 7])
    cp_b2 = cp(b2_hbm, b2_v, sem.at[NC + 8])
    for c_ in (cp_wk, cp_gw, cp_x[0], cp_x[1], cp_wq, *cp_x[2:], cp_w1, cp_b1, cp_b2, cp_wv, cp_wo, cp_w2):
        c_.start()

    ties = []
    mean, held = {}, {}
    zacc = [None]

    def tie(v):
        ties.append(v if v.dtype == u32 else pltpu.bitcast(v, u32))

    def take(n):
        mine = ties[:n]
        del ties[:n]
        return mine

    def w_transpose(h, tied):
        for j in range(4 * h, 4 * h + 4):
            pk = _pk(wqk_v[:, j * 128:(j + 1) * 128].T)
            wqkT_p[j * 64:(j + 1) * 64, :] = pk
            if tied:
                for kk in range(8):
                    for jj in range(4):
                        tie(pk[8 * kk:8 * kk + 8, jj * 128:(jj + 1) * 128])

    def ext_rows():
        gw = jnp.broadcast_to(gw_v[...].astype(f32).reshape(1, D), (16, D))
        ri = lax.broadcasted_iota(jnp.int32, (16, D), 0)
        return jnp.where(ri == 0, gw, jnp.where(ri == 1, 1.0 / D, 0.0))

    def use_ext(e, t):
        gate_v[:, t * 128:(t + 1) * 128] = jnp.broadcast_to(jax.nn.sigmoid(e[0:1, :]), (8, 128))
        mean[t] = e[1:2, :]

    def qk_dot(c, h, nties=0, off=0):
        if nties:
            slots = {}
            for tv, sidx in zip(take(nties), _spread(nties, 128, off)):
                slots.setdefault((sidx // 4, sidx % 4), []).append(tv)
            lhs = _tie_rows(lambda m0, m1, j: wqkT_p[h * 256 + m0 * 8:h * 256 + m1 * 8, j * 128:(j + 1) * 128],
                            32, 4, slots, tmask)
        else:
            lhs = _upk(wqkT_p[h * 256:(h + 1) * 256, :])
        if h == 1:
            lhs = jnp.concatenate([lhs, _upk(wqkT_p[512:520, :])], axis=0)
        return _dot_nt(lhs, x_v[c * TC:(c + 1) * TC, :])

    def q_store(c, q):
        pq_p[:, c * TC:(c + 1) * TC] = _pk(q.astype(bf16))

    def k_finish(c, pe, po):
        pkT_p[:, c * TC:c * TC + 128] = _pk(pe.astype(bf16))
        pkT_p[:, c * TC + 128:(c + 1) * TC] = _pk(po.astype(bf16))
        s = pe + po
        zacc[0] = s if zacc[0] is None else zacc[0] + s

    def k_store(c, k):
        for par in range(2):
            use_ext(k[D:D + 8, par * 128:(par + 1) * 128], 2 * c + par)
        pk = _phi(k[:D])
        k_finish(c, pk[:, :128], pk[:, 128:])

    def layernorm(c):
        xT, stats = {}, {}
        for par in range(2):
            t = 2 * c + par
            ts = slice(t * 128, (t + 1) * 128)
            for j in range(4):
                xT[par, j] = x_v[ts, j * 128:(j + 1) * 128].T
            m = mean.pop(t)
            vs = None
            for j in range(4):
                xc = xT[par, j].astype(f32) - m
                v = jnp.sum((xc * xc).reshape(16, 8, 128), axis=0)
                vs = v if vs is None else vs + v
                tie(vs)
            stats[par] = (m, lax.rsqrt(jnp.sum(vs, axis=0, keepdims=True) * (1.0 / D) + 1e-5))
        (me, re), (mo, ro) = stats[0], stats[1]
        for b in range(2):
            for r in range(0, 128, 16):
                rs = slice(r, r + 16)
                a11 = (xT[0, b][rs].astype(f32) - me) * re
                a21 = (xT[0, 2 + b][rs].astype(f32) - me) * re
                a12 = (xT[1, b][rs].astype(f32) - mo) * ro
                a22 = (xT[1, 2 + b][rs].astype(f32) - mo) * ro
                for i, l in enumerate(_lsums(a11, a12, a21, a22)):
                    pk = _pk(l.astype(bf16))
                    hL_p[i, (b * 128 + r) // 2:(b * 128 + r + 16) // 2, c * 128:(c + 1) * 128] = pk
                    tie(pk)

    def pk_ops(c):
        for r in range(0, HD, 64):
            def blk(par, half):
                u0 = (half * HD + r) // 2
                return (_upk(pkT_p[u0:u0 + 32, c * TC + par * 128:c * TC + (par + 1) * 128]).astype(f32)
                        * zi_v[half * HD + r:half * HD + r + 64, :])
            for i, l in enumerate(_lsums(blk(0, 0), blk(1, 0), blk(0, 1), blk(1, 1))):
                pk = _pk(l.astype(bf16))
                pkL_p[i, r // 2:r // 2 + 32, c * 128:(c + 1) * 128] = pk
                for k in range(4):
                    tie(pk[8 * k:8 * k + 8, :])

    TM = {}

    def t_piece(n, nties):
        def quad(par, col):
            return lambda: jnp.concatenate(
                [x_v[(2 * t + par) * 128:(2 * t + par + 1) * 128, col * HD:(col + 1) * HD] for t in range(NC)], axis=0)
        p = ORDER[n]
        R = _rhs_ops(quad(0, 0), quad(0, 1), quad(1, 0), quad(1, 1))
        TM[p] = _dot(_tie_value(_upk(pkL_p[p - 1]), take(nties), tmask), R[p]())
        if n == 6:
            C11, C12, C21, C22 = _combine(TM)
            tb_p[0:HD // 2, :] = _pk(jnp.concatenate([C11, C12], axis=1).astype(bf16))
            tb_p[HD // 2:, :] = _pk(jnp.concatenate([C21, C22], axis=1).astype(bf16))

    def u_stage(j, nties=0):
        def quad(par, col):
            return lambda: jnp.concatenate(
                [w1_v[(2 * t + par) * 128:(2 * t + par + 1) * 128, j * 256 + col * 128:j * 256 + (col + 1) * 128]
                 for t in range(NC)], axis=0)
        R = _rhs_ops(quad(0, 0), quad(0, 1), quad(1, 0), quad(1, 1))
        C11, C12, C21, C22 = _strassen(lambda i: _upk(hL_p[i]), lambda p: R[p](), _dot, take(nties), tmask)

        def gl(v, f0):
            return jax.nn.gelu(v + b1[:, f0:f0 + 128], approximate=True)
        G = (gl(C11, j * 256), gl(C12, j * 256 + 128), gl(C21, j * 256), gl(C22, j * 256 + 128))
        for i, l in enumerate(_lsums(*G)):
            gL_p[i, :, j * 128:(j + 1) * 128] = _pk(l.astype(bf16))

    def norm_stage(c):
        nb = {}
        for par in range(2):
            ts = slice((2 * c + par) * 128, (2 * c + par + 1) * 128)
            for b in range(4):
                pq = _upk(pq_p[b * 64:(b + 1) * 64, ts]).astype(f32)
                pq = _phi(pq)
                t3 = (pq * zb_v[b * 128:(b + 1) * 128, :]).reshape(8, DH, 128)
                den = jnp.sum(t3, axis=1, keepdims=True) + 1e-6
                nb[par, b] = (t3 * _rcp(den)).reshape(128, 128)
        ops = [[None, None] for _ in range(7)]
        for bp in range(2):
            for i, l in enumerate(_lsums(nb[0, bp], nb[1, bp], nb[0, 2 + bp], nb[1, 2 + bp])):
                ops[i][bp] = l.astype(bf16)
        R = [jnp.concatenate(o, axis=0) for o in ops]
        for p in ORDER:
            pk = _pk(R[RIDX[p]])
            for k in range(16):
                tie(pk[8 * k:8 * k + 8, :])
        held[c] = R

    def a_stage(c):
        R = held.pop(c)
        C = _strassen(lambda i: _upk(mL_p[i]), lambda p: R[RIDX[p]])
        aT = jnp.concatenate([jnp.concatenate([C[0], C[1]], axis=1), jnp.concatenate([C[2], C[3]], axis=1)], axis=0)
        cs = slice(c * TC, (c + 1) * TC)
        ga_v[:, cs] = gate_v[0:1, cs] * aT

    cp_wk.wait()
    w_transpose(1, tied=False)
    cp_x[0].wait()
    cp_gw.wait()
    g8 = wqk_v[0:16, D:D + 128].astype(f32)[0:8, :]
    tmask = (g8 >= 0.0) | (g8 < 0.0) | (g8 != g8)
    wqkT_p[512:520, :] = _pk(ext_rows().astype(bf16))
    k_store(0, qk_dot(0, 1))
    cp_x[1].wait()
    k_store(1, qk_dot(1, 1))
    cp_wq.wait()
    cp_x[2].wait()
    w_transpose(0, tied=True)
    k_store(2, qk_dot(2, 1, 128, 64))
    nxt = [0]

    def need(n):
        while len(ties) < n and nxt[0] < min(NC, nxt[1]):
            layernorm(nxt[0])
            nxt[0] += 1
    nxt.append(3)
    q_store(0, qk_dot(0, 0))
    q_store(1, qk_dot(1, 0))
    q2 = qk_dot(2, 0)
    for c in range(3, NC):
        cp_x[c].wait()
    q_store(2, q2)
    for c, n in zip(range(3, NC), (0,) + TK[:4]):
        need(n)
        k_store(c, qk_dot(c, 1, min(n, len(ties))))
        nxt[1] = c + 1
    z = jnp.broadcast_to(jnp.sum(zacc[0], axis=1, keepdims=True), (D, 128))
    zb_v[...] = z
    zi_v[...] = _rcp(z)
    keep = list(ties)
    del ties[:]
    for c in range(NC):
        pk_ops(c)
    lop = list(ties)
    del ties[:]
    ties.extend(keep)
    for j, (c, n) in enumerate(zip(range(3, NC), TK[4:9])):
        need(n)
        m = LT[j]
        mine = take(min(n, len(ties)))
        ties[:0] = lop[:m] + mine
        lop = lop[m:]
        q_store(c, qk_dot(c, 0, m + len(mine), 48 if j == 0 else 0))
    assert not lop
    for n, nt in enumerate(TK[9:]):
        need(nt)
        t_piece(n, nt)
    assert nxt[0] == NC and not ties

    for c_ in (cp_w1, cp_b1, cp_b2, cp_wv, cp_wo):
        c_.wait()
    for j in range(4):
        woT_p[j * 64:(j + 1) * 64, :] = _pk(wo_v[:, j * 128:(j + 1) * 128].T)
    b1 = b1_v[...].astype(f32).reshape(1, F)
    u_stage(0)
    msk = (lax.broadcasted_iota(jnp.int32, (128, 128), 0) // DH) == (lax.broadcasted_iota(jnp.int32, (128, 128), 1) // DH)
    kvs = []
    for b in range(4):
        kv = _dot(_upk(tb_p[b * 64:(b + 1) * 64, :]), wv_v[:, b * 128:(b + 1) * 128])
        kvs.append(jnp.where(msk, kv, 0.0).astype(bf16))
    u_stage(1)
    Ms = [_dot_nt(_upk(woT_p[:, b * 128:(b + 1) * 128]), kvs[b]) for b in range(4)]
    for bp in range(2):
        for i, l in enumerate(_lsums(Ms[bp][:HD], Ms[2 + bp][:HD], Ms[bp][HD:], Ms[2 + bp][HD:])):
            mL_p[i, :, bp * 128:(bp + 1) * 128] = _pk(l.astype(bf16))
    for j in (2, 3, 4):
        norm_stage(2 * j - 4)
        norm_stage(2 * j - 3)
        u_stage(j, 224)
        a_stage(2 * j - 4)
        a_stage(2 * j - 3)
    norm_stage(6)
    norm_stage(7)
    u_stage(5, 224)
    a_stage(6)
    u_stage(6)
    a_stage(7)

    cp_w2.wait()
    b2f_v[...] = jnp.broadcast_to(b2_v[...].astype(f32).reshape(1, S), (8, S))

    def out_tile(tt, obT, s):
        o_v[tt, :] = obT
        cp(o_v.at[tt, :], out_hbm.at[0, tt, :], s).start()

    pend_p[...] = jnp.zeros((HD, 128), u32)

    def y_body(i, carry):
        tprev = pl.multiple_of(jnp.where(i == 0, 14, 4 * i - 2) * 128, 128)
        out_tile(pl.ds(tprev, 128), _upk(pend_p[...]).T, sem_o.at[jnp.where(i == 0, 1, 0)])
        for k in range(2):
            c0 = pl.multiple_of((2 * i + k) * TC, TC)

            def quad(par, col):
                return lambda: jnp.concatenate(
                    [w2_v[(2 * t + par) * 128:(2 * t + par + 1) * 128, pl.ds(c0 + col * 128, 128)] for t in range(NF)],
                    axis=0)
            R = _rhs_ops(quad(0, 0), quad(0, 1), quad(1, 0), quad(1, 1))
            Y11, Y12, Y21, Y22 = _strassen(lambda n: _upk(gL_p[n]), lambda p: R[p]())
            for par, (Ya, Yb) in ((1, (Y12, Y22)), (0, (Y11, Y21))):
                tt = pl.ds(c0 + par * 128, 128)
                y = jnp.concatenate([Ya, Yb], axis=0) + b2f_v[0:1, tt]
                oT = (ga_v[:, tt] + (1.0 - gate_v[0:1, tt]) * y).astype(bf16)
                if k == 1 and par == 0:
                    pend_p[...] = _pk(oT)
                else:
                    out_tile(tt, oT.T, sem_o.at[0])
        return carry
    lax.fori_loop(0, NC // 2, y_body, 0)
    t14 = pl.ds(14 * 128, 128)
    cp(o_v.at[t14, :], out_hbm.at[0, t14, :], sem_o.at[1]).wait()
    out_tile(t14, _upk(pend_p[...]).T, sem_o.at[0])
    cp(o_v, out_hbm.at[0], sem_o.at[0]).wait()


@jax.jit
def pallas_gated_mix__linear_attn_block__mixer_token_mlp__prompt_kernel(
        A_x, A_wqkv, A_wo, B_x, B_w1, B_b1, B_w2, B_b2, gate_w):
    del B_x
    assert A_x.shape == (1, S, D) and B_w1.shape == (S, F) and B_w2.shape == (F, S), "fixed problem shape"
    vm = pltpu.VMEM
    scratch = [
        vm((S, D), bf16),
        vm((D, 2 * D), bf16),
        vm((D, D), bf16),
        vm((D, D), bf16),
        vm((S, F), bf16),
        vm((F, S), bf16),
        vm((S, D), bf16),
        vm((F,), bf16),
        vm((S,), bf16),
        vm((D,), bf16),
        vm((D + 8, D), u32),
        vm((7, D // 4, S // 2), u32),
        vm((HD, S), u32),
        vm((HD, S), u32),
        vm((7, D // 4, S // 2), u32),
        vm((D, 128), f32),
        vm((HD, D), u32),
        vm((HD, D), u32),
        vm((7, D // 4, HD), u32),
        vm((7, D // 4, F // 2), u32),
        vm((8, S), f32),
        vm((D, 128), f32),
        vm((D, S), f32),
        vm((8, S), f32),
        vm((HD, 128), u32),
        pltpu.SemaphoreType.DMA((NC + 9,)),
        pltpu.SemaphoreType.DMA((2,)),
    ]
    any_spec = pl.BlockSpec(memory_space=pl.ANY)
    return pl.pallas_call(
        _kernel,
        out_shape=jax.ShapeDtypeStruct((1, S, D), bf16),
        in_specs=[any_spec] * 8,
        out_specs=any_spec,
        scratch_shapes=scratch,
        compiler_params=pltpu.CompilerParams(
            vmem_limit_bytes=100 * 1024 * 1024, disable_semaphore_checks=True, disable_bounds_checks=True),
    )(A_x, A_wqkv, A_wo, B_w1, B_w2, B_b1, B_b2, gate_w)
```
